```python
import jax
import jax.numpy as jnp

def _softmax(x, axis=-1):
    return jax.nn.softmax(x, axis=axis)
def _gelu(x):
    return jax.nn.gelu(x, approximate=True)
def _silu(x):
    return jax.nn.silu(x)
def _sigmoid(x):
    return jax.nn.sigmoid(x)
def _layernorm(x, axis=-1, eps=1e-5):
    m = jnp.mean(x, axis=axis, keepdims=True)
    v = jnp.var(x, axis=axis, keepdims=True)
    return (x - m) / jnp.sqrt(v + eps)
def _scatter_add(tgt, idx, src, axis=0):
    return tgt.at[idx].add(src)
def _segment_sum(src, seg, n):
    return jax.ops.segment_sum(src, seg, n)
class _Rng:
    def __init__(self, key):
        self._k = key
    def _next(self):
        self._k, sub = jax.random.split(self._k)
        return sub
    def normal(self, shape):
        return jax.random.normal(self._next(), shape, dtype=jnp.bfloat16)
    def randint(self, lo, hi, shape):
        return jax.random.randint(self._next(), shape, lo, hi, dtype=jnp.int32)
    def uniform(self, shape, lo=0.0, hi=1.0):
        return jax.random.uniform(self._next(), shape, jnp.bfloat16, lo, hi)
    def permutation(self, n):
        return jax.random.permutation(self._next(), n)


kernel_name = 'gated_mix__compressed_kv_cla__ssm_conv_s5__prompt'

def setup_inputs():
    _rng = _Rng(jax.random.key(int.from_bytes(__import__("os").urandom(4), "little")))
    _w = (lambda a: (lambda t: t.astype(jnp.bfloat16) if jnp.issubdtype(t.dtype, jnp.floating) else t)(jnp.asarray(a)))
    def _A_setup():
        B, H, Sq, Sk, D, M = 1, 16, 2048, 2048, 256, 448
        Dc = 4 * D
        return {
            "x": _w((lambda *s: _rng.normal(s) * 0.05)(B, Sq, M)),
            "c_kv": _w((lambda *s: _rng.normal(s) * 0.05)(B, Sk, Dc)),
            "w_q": _w((lambda *s: _rng.normal(s) * 0.05)(M, H, D) * (M ** -0.5)),
            "w_uk": _w((lambda *s: _rng.normal(s) * 0.05)(Dc, H, D) * (Dc ** -0.5)),
            "w_uv": _w((lambda *s: _rng.normal(s) * 0.05)(Dc, H, D) * (Dc ** -0.5)),
            "w_o": _w((lambda *s: _rng.normal(s) * 0.05)(H, D, M) * ((H * D) ** -0.5)),
        }
    _A_in = _A_setup()

    def _B_setup():
        B, S, D = 1, 2048, 448
        P = D
        Lambda_re = -0.5 * jnp.exp((lambda *s: _rng.normal(s) * 0.05)(P))
        Lambda_im = (lambda *s: _rng.normal(s) * 0.05)(P) * 1.0
        B_re = (lambda *s: _rng.normal(s) * 0.05)(P, D) * (D ** -0.5)
        B_im = (lambda *s: _rng.normal(s) * 0.05)(P, D) * (D ** -0.5)
        C_re = (lambda *s: _rng.normal(s) * 0.05)(D, P) * (P ** -0.5)
        C_im = (lambda *s: _rng.normal(s) * 0.05)(D, P) * (P ** -0.5)
        log_dt = (lambda *s: _rng.normal(s) * 0.05)(P) * 0.3 - 2.0
        Dskip = (lambda *s: _rng.normal(s) * 0.05)(D)
        return {
            "x": _w((lambda *s: _rng.normal(s) * 0.05)(B, S, D)),
            "Lambda_re": _w(Lambda_re),
            "Lambda_im": _w(Lambda_im),
            "B_re": _w(B_re),
            "B_im": _w(B_im),
            "C_re": _w(C_re),
            "C_im": _w(C_im),
            "log_dt": _w(log_dt),
            "Dskip": _w(Dskip),
        }
    _B_in = _B_setup()

    return {
        "A_x": _A_in["x"],
        "A_c_kv": _A_in["c_kv"],
        "A_w_q": _A_in["w_q"],
        "A_w_uk": _A_in["w_uk"],
        "A_w_uv": _A_in["w_uv"],
        "A_w_o": _A_in["w_o"],
        "B_x": _B_in["x"],
        "B_Lambda_re": _B_in["Lambda_re"],
        "B_Lambda_im": _B_in["Lambda_im"],
        "B_B_re": _B_in["B_re"],
        "B_B_im": _B_in["B_im"],
        "B_C_re": _B_in["C_re"],
        "B_C_im": _B_in["C_im"],
        "B_log_dt": _B_in["log_dt"],
        "B_Dskip": _B_in["Dskip"],
        "gate_w": _w((lambda *s: _rng.normal(s) * 0.05)(448)),
    }

def reference(A_x, A_c_kv, A_w_q, A_w_uk, A_w_uv, A_w_o, B_x, B_Lambda_re, B_Lambda_im, B_B_re, B_B_im, B_C_re, B_C_im, B_log_dt, B_Dskip, gate_w):
    def _A_ref(x, c_kv, w_q, w_uk, w_uv, w_o):
        B, Sq, M = x.shape[0], x.shape[1], x.shape[2]
        Sk = c_kv.shape[1]
        H, D = w_q.shape[1], w_q.shape[2]
        q = jnp.einsum("bqm,mhd->bhqd", x, w_q)
        k = jnp.einsum("bkc,chd->bhkd", c_kv, w_uk)
        v = jnp.einsum("bkc,chd->bhkd", c_kv, w_uv)
        scores = jnp.einsum("bhqd,bhkd->bhqk", q, k) * (D ** -0.5)
        off = Sk - Sq
        qi = jnp.arange(Sq)[:, None]
        kj = jnp.arange(Sk)[None, :]
        cmask = kj <= (qi + off)
        scores = jnp.where(cmask[None, None], scores, -1e9)
        p = _softmax(scores, axis=-1)
        ctx = jnp.einsum("bhqk,bhkd->bhqd", p, v)
        return jnp.einsum("bhqd,hdm->bqm", ctx, w_o)

    def _B_ref(x, Lambda_re, Lambda_im, B_re, B_im, C_re, C_im, log_dt, Dskip):
        Bsz, L, H = x.shape
        Lam = Lambda_re + 1j * Lambda_im
        Bmat = B_re + 1j * B_im
        Cmat = C_re + 1j * C_im
        dt = jnp.exp(log_dt)
        Lam_bar = jnp.exp(dt * Lam)
        B_bar = ((Lam_bar - 1.0) / Lam)[:, None] * Bmat
        Bu = jnp.einsum("bld,pd->blp", x + 0j, B_bar)
        h = jnp.zeros_like(Bu[:, 0, :])
        hs = []
        for t in range(L):
            h = Lam_bar[None, :] * h + Bu[:, t, :]
            hs.append(h)
        hseq = jnp.stack(hs, 1)
        y = 2.0 * jnp.einsum("blp,dp->bld", hseq, Cmat).real + x * Dskip[None, None, :]
        return y

    x = A_x
    g = _sigmoid((x * gate_w).sum(-1, keepdims=True))
    a = _A_ref(x, A_c_kv, A_w_q, A_w_uk, A_w_uv, A_w_o)
    b = _B_ref(x, B_Lambda_re, B_Lambda_im, B_B_re, B_B_im, B_C_re, B_C_im, B_log_dt, B_Dskip)
    return g * a + (1 - g) * b
```

```python
import functools
import jax
import jax.numpy as jnp
import numpy as np
import jax.experimental.pallas as pl
import jax.experimental.pallas.tpu as pltpu

S = 2048
M = 448
H = 16
D = 256
DC = 1024
NCH = 16
TCH = S // NCH
PITCH = TCH + 4
LOG2E = 1.4426950408889634
NT = (((1,), (1,)), ((), ()))
F32 = jnp.float32
BF16 = jnp.bfloat16
U32 = jnp.uint32


def _dot(a, b):
    return jnp.dot(a, b, preferred_element_type=F32)


def _dot_nt(a, b):
    return jax.lax.dot_general(a, b, NT, preferred_element_type=F32)


def _cmul(ar, ai, br, bi):
    return ar * br - ai * bi, ar * bi + ai * br


def _tiles(v, sign):
    t = [v[:, j * 128:(j + 1) * 128] for j in range(3)]
    t.append(jnp.concatenate([v[:, 384:], sign * v[:, 384:]], axis=1))
    return t


def _ssm(xt_ref, x_ref, lre_ref, lim_ref, bre_ref, bim_ref, cre_ref, cim_ref, ldt_ref, dsk_ref, gw_ref,
         b_ref, g_ref, hre_ref, him_ref, pre_u, pre_y):
    lre = lre_ref[...].astype(F32).reshape(1, M)
    lim = lim_ref[...].astype(F32).reshape(1, M)
    dt = jnp.exp(ldt_ref[...].astype(F32).reshape(1, M)).astype(BF16).astype(F32)
    mag = jnp.exp(dt * lre)
    ang = dt * lim
    ar = mag * jnp.cos(ang)
    ai = mag * jnp.sin(ang)
    den = lre * lre + lim * lim
    cr = _tiles(((ar - 1.0) * lre + ai * lim) / den, 1.0)
    ci = _tiles((ai * lre - (ar - 1.0) * lim) / den, -1.0)
    RB = 512
    pre_u(0)
    bre = bre_ref[...]
    bim = bim_ref[...]
    bcat = jnp.concatenate([bre[:384], bim[:384], bre[384:], bim[384:]], axis=0)
    for r in range(S // RB):
        rows = pl.ds(r * RB, RB)
        if r > 0:
            pre_u(r)
        xb = xt_ref[:, rows].T
        x_ref[rows, :] = xb
        u = _dot_nt(xb, bcat)
        for j in range(4):
            if j < 3:
                ur = u[:, j * 128:(j + 1) * 128]
                ui = u[:, 384 + j * 128:384 + (j + 1) * 128]
            else:
                ur = u[:, 768:]
                ui = pltpu.roll(ur, 64, 1)
            br, bi = _cmul(cr[j], ci[j], ur, ui)
            for cc in range(RB // TCH):
                dst = pl.ds((r * (RB // TCH) + cc) * PITCH, TCH)
                hre_ref[j, dst, :] = br[cc * TCH:(cc + 1) * TCH]
                him_ref[j, dst, :] = bi[cc * TCH:(cc + 1) * TCH]
    A_r = [jnp.broadcast_to(v, (NCH, 128)) for v in _tiles(ar, 1.0)]
    A_i = [jnp.broadcast_to(v, (NCH, 128)) for v in _tiles(ai, -1.0)]

    def mul_state(Ar, Ai, st):
        o = [_cmul(Ar[j], Ai[j], st[0][j], st[1][j]) for j in range(4)]
        return [a for a, _ in o], [b for _, b in o]

    def load(t):
        idx = pl.ds(t, NCH, stride=PITCH)
        return [hre_ref[j, idx, :] for j in range(4)], [him_ref[j, idx, :] for j in range(4)]

    def add(a, b):
        return [p + q for p, q in zip(a[0], b[0])], [p + q for p, q in zip(a[1], b[1])]

    def step1(t, st):
        return add(mul_state(A_r, A_i, st), load(t))

    z = jnp.zeros((NCH, 128), F32)
    end = jax.lax.fori_loop(0, TCH, step1, ([z] * 4, [z] * 4), unroll=8)
    Pr, Pi = A_r, A_i

    def square(Pr, Pi):
        return [a * a - b * b for a, b in zip(Pr, Pi)], [2.0 * a * b for a, b in zip(Pr, Pi)]

    for _ in range(int(np.log2(TCH))):
        Pr, Pi = square(Pr, Pi)
    row = jax.lax.broadcasted_iota(jnp.int32, (NCH, 128), 0)

    def shift(st, k):
        f = lambda v: jnp.where(row >= k, pltpu.roll(v, k, 0), 0.0)
        return [f(v) for v in st[0]], [f(v) for v in st[1]]

    car = shift(end, 1)
    k = 1
    while k < NCH:
        car = add(car, mul_state(Pr, Pi, shift(car, k)))
        Pr, Pi = square(Pr, Pi)
        k *= 2

    def step2(t, st):
        st = add(mul_state(A_r, A_i, st), load(t))
        idx = pl.ds(t, NCH, stride=PITCH)
        for j in range(4):
            hre_ref[j, idx, :] = st[0][j]
        for j in range(3):
            him_ref[j, idx, :] = st[1][j]
        return st

    jax.lax.fori_loop(0, TCH, step2, car, unroll=8)
    dsk = jnp.broadcast_to(dsk_ref[...].astype(F32).reshape(1, M), (128, M)).T
    gw = jnp.broadcast_to(gw_ref[...].astype(F32).reshape(1, M), (128, M)).T
    dsk = jnp.concatenate([dsk] * (RB // 128), axis=1)
    gw = jnp.concatenate([gw] * (RB // 128), axis=1)
    pre_y()
    cre = cre_ref[...]
    cim = cim_ref[...]
    ccat = jnp.concatenate([cre[:, :384], -cim[:, :384], cre[:, 384:], -cim[:, 384:]], axis=1)
    for r in range(S // RB):
        rows = pl.ds(r * RB, RB)
        def ld(ref, j):
            return jnp.concatenate([ref[j, pl.ds((r * (RB // TCH) + cc) * PITCH, TCH), :].astype(BF16)
                                    for cc in range(RB // TCH)], axis=0)
        hcat = jnp.concatenate([ld(hre_ref, j) for j in range(3)] + [ld(him_ref, j) for j in range(3)]
                               + [ld(hre_ref, 3)], axis=1)
        xf = xt_ref[:, rows].astype(F32)
        y = 2.0 * _dot_nt(ccat, hcat) + xf * dsk
        g = jax.nn.sigmoid(jnp.sum(xf * gw, axis=0, keepdims=True))
        b_ref[:, rows] = (1.0 - g) * y
        g_ref[rows, :] = jnp.broadcast_to(g, (128, RB)).T


def _kernel(xt_hbm, c_hbm, wq_hbm, wk_hbm, wv_hbm, wo_hbm, bre_hbm, bim_hbm, cre_hbm, cim_hbm,
            lre_ref, lim_ref, ldt_ref, dsk_ref, gw_ref,
            o_hbm,
            xt_ref, x_ref, c_ref, wq_buf, wk_buf, wv_buf, wo_buf, bc_buf, sems, osem,
            q_s, k_s, v_s, ctx_s, acc_ref, g_ref, hre_ref, him_ref, *, BQ, PRB, DIAG, ORDER):
    def wcopies(w_hbm, buf, i):
        wu = w_hbm.bitcast(U32)
        return [pltpu.make_async_copy(wu.at[:, pl.ds(128 * j, 128)], buf.at[j], sems.at[i + j]) for j in range(2)]

    cp_x = [pltpu.make_async_copy(xt_hbm.at[0, :, pl.ds(512 * r, 512)], xt_ref.at[:, pl.ds(512 * r, 512)],
                                  sems.at[r]) for r in range(4)]
    cp_bc = [pltpu.make_async_copy(w, bc_buf.at[j], sems.at[4 + j])
             for j, w in enumerate((bre_hbm, bim_hbm, cre_hbm, cim_hbm))]
    cp_q = wcopies(wq_hbm, wq_buf, 8)
    rest = ([pltpu.make_async_copy(c_hbm.at[0], c_ref, sems.at[10])]
            + wcopies(wk_hbm, wk_buf, 11) + wcopies(wv_hbm, wv_buf, 13)
            + [pltpu.make_async_copy(wo_hbm, wo_buf, sems.at[15])])
    for cp in (cp_x[0], cp_bc[0], cp_bc[1]):
        cp.start()

    def pre_u(r):
        if r == 0:
            for cp in (cp_x[0], cp_bc[0], cp_bc[1]):
                cp.wait()
            for cp in cp_x[1:] + cp_bc[2:]:
                cp.start()
        else:
            cp_x[r].wait()
        if r == 1:
            for cp in cp_q:
                cp.start()
        if r == 2:
            for cp in rest:
                cp.start()

    def pre_y():
        cp_bc[2].wait()
        cp_bc[3].wait()

    _ssm(xt_ref, x_ref, lre_ref, lim_ref, bc_buf.at[0], bc_buf.at[1], bc_buf.at[2], bc_buf.at[3],
         ldt_ref, dsk_ref, gw_ref, acc_ref, g_ref, hre_ref, him_ref, pre_u, pre_y)
    for cp in cp_q:
        cp.wait()

    def qproj(p, carry):
        w = jnp.concatenate([wq_buf[j, pl.ds(p, M, stride=8), :] for j in range(2)], axis=1)
        w2 = jnp.concatenate([pltpu.bitcast(w << 16, F32).astype(BF16),
                              pltpu.bitcast(w & jnp.uint32(0xFFFF0000), F32).astype(BF16)], axis=1)
        for r in range(S // 1024):
            rows = pl.ds(r * 1024, 1024)
            q2 = (_dot(x_ref[rows, :], w2) * (LOG2E / 16.0)).astype(BF16)
            q_s[2 * p, rows, :] = q2[:, :D]
            q_s[2 * p + 1, rows, :] = q2[:, D:]
        return carry

    jax.lax.fori_loop(0, H // 2, qproj, 0)
    for cp in rest:
        cp.wait()

    def ocopy(i):
        cols = pl.ds(i * BQ, BQ)
        return pltpu.make_async_copy(acc_ref.at[:, cols], o_hbm.at[0, :, cols], osem.at[i])

    def head(h, carry):
        pair = h // 2
        sh = ((1 - h % 2) * 16).astype(U32)

        def unpack(buf, n):
            w = jnp.concatenate([buf[j, pl.ds(pair, n, stride=8), :] for j in range(2)], axis=1)
            return pltpu.bitcast((w << sh) & jnp.uint32(0xFFFF0000), F32).astype(BF16)

        wk = unpack(wk_buf, DC)
        wv = unpack(wv_buf, DC)
        NB = S // BQ
        HB = BQ // 2

        def proj(r):
            rows = pl.ds(r * PRB, PRB)
            k_s[rows, :] = _dot(c_ref[rows, :], wk).astype(BF16)
            v_s[rows, :] = _dot(c_ref[rows, :], wv).astype(BF16)

        def tri(n):
            ri = jax.lax.broadcasted_iota(jnp.int32, (n, n), 0)
            ci = jax.lax.broadcasted_iota(jnp.int32, (n, n), 1)
            return ci <= ri

        def qk(i):
            r0 = i * BQ
            if not DIAG:
                return (_dot_nt(q_s[h, pl.ds(r0, BQ), :], k_s[pl.ds(0, r0 + BQ), :]),)
            return (_dot_nt(q_s[h, pl.ds(r0, BQ), :], k_s[pl.ds(0, r0 + HB), :]),
                    _dot_nt(q_s[h, pl.ds(r0 + HB, HB), :], k_s[pl.ds(r0 + HB, HB), :]))

        def msk(s, n):
            sd = jnp.where(tri(n), s[:, -n:], -1e9)
            return sd if s.shape[1] == n else jnp.concatenate([s[:, :-n], sd], axis=1)

        def soft(s, r0):
            m = jnp.max(s, axis=1, keepdims=True)
            p = jnp.exp2(s - m)
            sc = g_ref[pl.ds(r0, s.shape[0]), :] * (1.0 / jnp.sum(p, axis=1, keepdims=True))
            return p.astype(BF16), jnp.concatenate([sc, sc], axis=1)

        def sm(i, s):
            if not DIAG:
                return soft(msk(s[0], BQ), i * BQ)
            pt, lt = soft(msk(s[0][:HB], HB), i * BQ)
            pb, lb = soft(jnp.concatenate([s[0][HB:], msk(s[1], HB)], axis=1), i * BQ + HB)
            return (jnp.concatenate([pt, pb[:, :-HB]], axis=0), pb[:, -HB:]), (lt, lb)

        def pv(i, pl_):
            r0 = i * BQ
            p, l = pl_
            if not DIAG:
                return (_dot(p, v_s[pl.ds(0, r0 + BQ), :]) * l).astype(BF16)
            c = _dot(p[0], v_s[pl.ds(0, r0 + HB), :])
            cb = c[HB:] + _dot(p[1], v_s[pl.ds(r0 + HB, HB), :])
            return jnp.concatenate([(c[:HB] * l[0]).astype(BF16), (cb * l[1]).astype(BF16)], axis=0)

        def out(i, ctx):
            acc_ref[:, pl.ds(i * BQ, BQ)] += _dot_nt(wo_buf[h], ctx)

        acc_ref[:, pl.ds(S - BQ, BQ)] += _dot_nt(wo_buf[jnp.maximum(h - 1, 0)], ctx_s[...])
        for r in range(S // PRB):
            proj(r)
        c = None
        for i in range(NB):
            s = qk(i)
            if c is not None:
                out(i - 1, c)

                @pl.when(h == H - 1)
                def _():
                    ocopy(i - 1).start()
            c = pv(i, sm(i, s))
        ctx_s[...] = c
        return carry

    ctx_s[...] = jnp.zeros((BQ, D), BF16)
    jax.lax.fori_loop(0, H, head, 0)
    acc_ref[:, pl.ds(S - BQ, BQ)] += _dot_nt(wo_buf[H - 1], ctx_s[...])
    ocopy(S // BQ - 1).start()
    for i in range(S // BQ):
        ocopy(i).wait()


BQ = 256
PRB = 1024
DIAG = 1
ORDER = 8
flags = None


@jax.jit
def pallas_gated_mix__compressed_kv_cla__ssm_conv_s5__prompt_kernel(
      A_x, A_c_kv, A_w_q, A_w_uk, A_w_uv, A_w_o, B_x, B_Lambda_re, B_Lambda_im, B_B_re, B_B_im,
      B_C_re, B_C_im, B_log_dt, B_Dskip, gate_w):
    del B_x
    vm = pl.BlockSpec(memory_space=pltpu.VMEM)
    hbm = pl.BlockSpec(memory_space=pltpu.HBM)
    out = pl.pallas_call(
        functools.partial(_kernel, BQ=BQ, PRB=PRB, DIAG=DIAG, ORDER=ORDER),
        in_specs=[hbm] * 10 + [vm] * 5,
        out_specs=hbm,
        out_shape=jax.ShapeDtypeStruct((1, M, S), F32),
        scratch_shapes=[
            pltpu.VMEM((M, S), BF16),
            pltpu.VMEM((S, M), BF16),
            pltpu.VMEM((S, DC), BF16),
            pltpu.VMEM((2, M * 8, 128), U32),
            pltpu.VMEM((2, DC * 8, 128), U32),
            pltpu.VMEM((2, DC * 8, 128), U32),
            pltpu.VMEM((H, M, D), BF16),
            pltpu.VMEM((4, M, M), BF16),
            pltpu.SemaphoreType.DMA((16,)),
            pltpu.SemaphoreType.DMA((S // BQ,)),
            pltpu.VMEM((H, S, D), BF16),
            pltpu.VMEM((S, D), BF16),
            pltpu.VMEM((S, D), BF16),
            pltpu.VMEM((BQ, D), BF16),
            pltpu.VMEM((M, S), F32),
            pltpu.VMEM((S, 128), F32),
            pltpu.VMEM((4, NCH * PITCH, 128), F32),
            pltpu.VMEM((4, NCH * PITCH, 128), F32),
        ],
        compiler_params=pltpu.CompilerParams(vmem_limit_bytes=100 * 1024 * 1024, flags=flags),
    )(jnp.swapaxes(A_x, 1, 2), A_c_kv, A_w_q.reshape(M * H, D), A_w_uk.reshape(DC * H, D),
      A_w_uv.reshape(DC * H, D), jnp.swapaxes(A_w_o, 1, 2),
      B_B_re, B_B_im, B_C_re, B_C_im, B_Lambda_re, B_Lambda_im, B_log_dt, B_Dskip, gate_w)
    return jnp.swapaxes(out, 1, 2)
```

```python
import jax
import jax.numpy as jnp
import numpy as np
import jax.experimental.pallas as pl
import jax.experimental.pallas.tpu as pltpu

S = 2048
M = 448
H = 16
D = 256
DC = 1024
NCH = 8
TCH = S // NCH
PITCH = TCH + 4
LOG2E = 1.4426950408889634
NT = (((1,), (1,)), ((), ()))
F32 = jnp.float32
BF16 = jnp.bfloat16
U32 = jnp.uint32


def _dot(a, b):
    return jnp.dot(a, b, preferred_element_type=F32)


def _dot_nt(a, b):
    return jax.lax.dot_general(a, b, NT, preferred_element_type=F32)


def _cmul(ar, ai, br, bi):
    return ar * br - ai * bi, ar * bi + ai * br


def _tiles(v, sign):
    t = [v[:, j * 128:(j + 1) * 128] for j in range(3)]
    t.append(jnp.concatenate([v[:, 384:], sign * v[:, 384:]], axis=1))
    return t


def _ssm(xt_ref, x_ref, lre_ref, lim_ref, bre_ref, bim_ref, cre_ref, cim_ref, ldt_ref, dsk_ref, gw_ref,
         b_ref, g_ref, hre_ref, him_ref, pre_u, pre_y, pre_q, qproj):
    lre = lre_ref[...].astype(F32).reshape(1, M)
    lim = lim_ref[...].astype(F32).reshape(1, M)
    dt = jnp.exp(ldt_ref[...].astype(F32).reshape(1, M)).astype(BF16).astype(F32)
    mag = jnp.exp(dt * lre)
    ang = dt * lim
    ar = mag * jnp.cos(ang)
    ai = mag * jnp.sin(ang)
    den = lre * lre + lim * lim
    cr = _tiles(((ar - 1.0) * lre + ai * lim) / den, 1.0)
    ci = _tiles((ai * lre - (ar - 1.0) * lim) / den, -1.0)
    RB = 512
    pre_u(0)
    bre = bre_ref[...]
    bim = bim_ref[...]
    bcat = jnp.concatenate([bre[:384], bim[:384], bre[384:], bim[384:]], axis=0)
    for r in range(S // RB):
        rows = pl.ds(r * RB, RB)
        if r > 0:
            pre_u(r)
        xb = xt_ref[:, rows].T
        x_ref[rows, :] = xb
        u = _dot_nt(xb, bcat)
        for j in range(4):
            if j < 3:
                ur = u[:, j * 128:(j + 1) * 128]
                ui = u[:, 384 + j * 128:384 + (j + 1) * 128]
            else:
                ur = u[:, 768:]
                ui = pltpu.roll(ur, 64, 1)
            br, bi = _cmul(cr[j], ci[j], ur, ui)
            for cc in range(RB // TCH):
                dst = pl.ds((r * (RB // TCH) + cc) * PITCH, TCH)
                hre_ref[j, dst, :] = br[cc * TCH:(cc + 1) * TCH]
                him_ref[j, dst, :] = bi[cc * TCH:(cc + 1) * TCH]
    A_r = [jnp.broadcast_to(v, (NCH, 128)) for v in _tiles(ar, 1.0)]
    A_i = [jnp.broadcast_to(v, (NCH, 128)) for v in _tiles(ai, -1.0)]

    def mul_state(Ar, Ai, st):
        o = [_cmul(Ar[j], Ai[j], st[0][j], st[1][j]) for j in range(4)]
        return [a for a, _ in o], [b for _, b in o]

    def load(t):
        idx = pl.ds(t, NCH, stride=PITCH)
        return [hre_ref[j, idx, :] for j in range(4)], [him_ref[j, idx, :] for j in range(4)]

    def add(a, b):
        return [p + q for p, q in zip(a[0], b[0])], [p + q for p, q in zip(a[1], b[1])]

    def step1(t, st):
        return add(mul_state(A_r, A_i, st), load(t))

    z = jnp.zeros((NCH, 128), F32)
    NQ = H // 4
    SPI = TCH // NQ

    def loop1(p, st):
        qproj(p)
        for t in range(SPI):
            st = step1(p * SPI + t, st)
        return st

    pre_q()
    end = jax.lax.fori_loop(0, NQ, loop1, ([z] * 4, [z] * 4))
    Pr, Pi = A_r, A_i

    def square(Pr, Pi):
        return [a * a - b * b for a, b in zip(Pr, Pi)], [2.0 * a * b for a, b in zip(Pr, Pi)]

    for _ in range(int(np.log2(TCH))):
        Pr, Pi = square(Pr, Pi)
    row = jax.lax.broadcasted_iota(jnp.int32, (NCH, 128), 0)

    def shift(st, k):
        f = lambda v: jnp.where(row >= k, pltpu.roll(v, k, 0), 0.0)
        return [f(v) for v in st[0]], [f(v) for v in st[1]]

    car = shift(end, 1)
    k = 1
    while k < NCH:
        car = add(car, mul_state(Pr, Pi, shift(car, k)))
        Pr, Pi = square(Pr, Pi)
        k *= 2

    def step2(t, st):
        st = add(mul_state(A_r, A_i, st), load(t))
        idx = pl.ds(t, NCH, stride=PITCH)
        for j in range(4):
            hre_ref[j, idx, :] = st[0][j]
        for j in range(3):
            him_ref[j, idx, :] = st[1][j]
        return st

    def loop2(p, st):
        qproj(NQ + p)
        for t in range(SPI):
            st = step2(p * SPI + t, st)
        return st

    jax.lax.fori_loop(0, NQ, loop2, car)
    dsk = jnp.broadcast_to(dsk_ref[...].astype(F32).reshape(1, M), (128, M)).T
    gw = jnp.broadcast_to(gw_ref[...].astype(F32).reshape(1, M), (128, M)).T
    dsk = jnp.concatenate([dsk] * (RB // 128), axis=1)
    gw = jnp.concatenate([gw] * (RB // 128), axis=1)
    pre_y()
    cre = cre_ref[...]
    cim = cim_ref[...]
    ccat = jnp.concatenate([cre[:, :384], -cim[:, :384], cre[:, 384:], -cim[:, 384:]], axis=1)
    for r in range(S // RB):
        rows = pl.ds(r * RB, RB)
        def ld(ref, j):
            return jnp.concatenate([ref[j, pl.ds((r * (RB // TCH) + cc) * PITCH, TCH), :].astype(BF16)
                                    for cc in range(RB // TCH)], axis=0)
        hcat = jnp.concatenate([ld(hre_ref, j) for j in range(3)] + [ld(him_ref, j) for j in range(3)]
                               + [ld(hre_ref, 3)], axis=1)
        xf = xt_ref[:, rows].astype(F32)
        y = 2.0 * _dot_nt(ccat, hcat) + xf * dsk
        g = jax.nn.sigmoid(jnp.sum(xf * gw, axis=0, keepdims=True))
        b_ref[:, rows] = (1.0 - g) * y
        g_ref[rows, :] = jnp.broadcast_to(g, (128, RB)).T


def _kernel(xt_hbm, c_hbm, wq_hbm, wk_hbm, wv_hbm, wo_hbm, bre_hbm, bim_hbm, cre_hbm, cim_hbm,
            lre_ref, lim_ref, ldt_ref, dsk_ref, gw_ref,
            o_hbm,
            xt_ref, x_ref, c_ref, wq_buf, wk_buf, wv_buf, wo_buf, bc_buf, sems, osem,
            q_s, k_s, v_s, ctx_s, ml_s, acc_ref, g_ref, hre_ref, him_ref):
    def wcopies(w_hbm, buf, i):
        wu = w_hbm.bitcast(U32)
        return [pltpu.make_async_copy(wu.at[:, pl.ds(128 * j, 128)], buf.at[j], sems.at[i + j]) for j in range(2)]

    cp_x = [pltpu.make_async_copy(xt_hbm.at[0, :, pl.ds(512 * r, 512)], xt_ref.at[:, pl.ds(512 * r, 512)],
                                  sems.at[r]) for r in range(4)]
    cp_bc = [pltpu.make_async_copy(w, bc_buf.at[j], sems.at[4 + j])
             for j, w in enumerate((bre_hbm, bim_hbm, cre_hbm, cim_hbm))]
    cp_q = wcopies(wq_hbm, wq_buf, 8)
    rest = ([pltpu.make_async_copy(c_hbm.at[0], c_ref, sems.at[10])]
            + wcopies(wk_hbm, wk_buf, 11) + wcopies(wv_hbm, wv_buf, 13)
            + [pltpu.make_async_copy(wo_hbm, wo_buf, sems.at[15])])
    for cp in (cp_x[0], cp_bc[0], cp_bc[1]):
        cp.start()

    def pre_u(r):
        if r == 0:
            for cp in (cp_x[0], cp_bc[0], cp_bc[1]):
                cp.wait()
            for cp in cp_x[1:]:
                cp.start()
        else:
            cp_x[r].wait()
        if r == 1:
            for cp in cp_q:
                cp.start()

    def pre_q():
        for cp in cp_q:
            cp.wait()
        for cp in cp_bc[2:] + rest:
            cp.start()

    def pre_y():
        cp_bc[2].wait()
        cp_bc[3].wait()

    def qproj(p):
        w = jnp.concatenate([wq_buf[j, pl.ds(p, M, stride=8), :] for j in range(2)], axis=1)
        w2 = jnp.concatenate([pltpu.bitcast(w << 16, F32).astype(BF16),
                              pltpu.bitcast(w & jnp.uint32(0xFFFF0000), F32).astype(BF16)], axis=1)
        for r in range(S // 1024):
            rows = pl.ds(r * 1024, 1024)
            q2 = (_dot(x_ref[rows, :], w2) * (LOG2E / 16.0)).astype(BF16)
            q_s[2 * p, rows, :] = q2[:, :D]
            q_s[2 * p + 1, rows, :] = q2[:, D:]

    _ssm(xt_ref, x_ref, lre_ref, lim_ref, bc_buf.at[0], bc_buf.at[1], bc_buf.at[2], bc_buf.at[3],
         ldt_ref, dsk_ref, gw_ref, acc_ref, g_ref, hre_ref, him_ref, pre_u, pre_y, pre_q, qproj)
    for cp in rest:
        cp.wait()

    def ocopy(i):
        cols = pl.ds(i * BQ, BQ)
        return pltpu.make_async_copy(acc_ref.at[:, cols], o_hbm.at[0, :, cols], osem.at[i])

    def kvproj(i, carry):
        for buf, dst in ((wk_buf, k_s), (wv_buf, v_s)):
            w = jnp.concatenate([buf[j, pl.ds(i, DC, stride=8), :] for j in range(2)], axis=1)
            ws = [(2 * i, pltpu.bitcast(w << 16, F32).astype(BF16)),
                  (2 * i + 1, pltpu.bitcast(w & jnp.uint32(0xFFFF0000), F32).astype(BF16))]
            for hh, wb in ws:
                for r in range(S // PRB):
                    rows = pl.ds(r * PRB, PRB)
                    dst[hh, rows, :] = _dot(c_ref[rows, :], wb).astype(BF16)
        return carry

    jax.lax.fori_loop(0, H // 2, kvproj, 0)

    def head(h, carry):
        NB = S // BQ
        HB = BQ // 2

        def tri(n):
            ri = jax.lax.broadcasted_iota(jnp.int32, (n, n), 0)
            ci = jax.lax.broadcasted_iota(jnp.int32, (n, n), 1)
            return ci <= ri

        def qk(i):
            r0 = i * BQ
            q = q_s[h, pl.ds(r0, BQ), :]
            ss = [_dot_nt(q, k_s[h, pl.ds(j * CW, CW), :]) for j in range(r0 // CW)]
            sa = _dot_nt(q, k_s[h, pl.ds(r0, HB), :])
            sb = _dot_nt(q_s[h, pl.ds(r0 + HB, HB), :], k_s[h, pl.ds(r0 + HB, HB), :])
            t = tri(HB)
            sa = jnp.concatenate([jnp.where(t, sa[:HB], -1e9), sa[HB:]], axis=0)
            sb = jnp.where(t, sb, -1e9)
            mx = sa
            for sj in ss:
                for u in range(CW // 128):
                    mx = jnp.maximum(mx, sj[:, u * 128:(u + 1) * 128])
            mx = jnp.concatenate([mx[:HB], jnp.maximum(mx[HB:], sb)], axis=0)
            m = jnp.broadcast_to(jnp.max(mx, axis=1, keepdims=True), (BQ, 128))
            ml_s[0] = m
            return ss, sa, sb

        def pv(i, st):
            r0 = i * BQ
            ss, sa, sb = st
            m = ml_s[0]
            pa = jnp.exp2(sa - m)
            pb = jnp.exp2(sb - m[HB:])
            ml_s[1] = jnp.concatenate([pa[:HB], pa[HB:] + pb], axis=0)
            c = _dot(pa.astype(BF16), v_s[h, pl.ds(r0, HB), :])
            c = jnp.concatenate([c[:HB], c[HB:] + _dot(pb.astype(BF16), v_s[h, pl.ds(r0 + HB, HB), :])], axis=0)
            for j, sj in enumerate(ss):
                m = ml_s[0]
                ps = [jnp.exp2(sj[:, u * 128:(u + 1) * 128] - m) for u in range(CW // 128)]
                l = ml_s[1]
                for p in ps:
                    l = l + p
                ml_s[1] = l
                c = c + _dot(jnp.concatenate(ps, axis=1).astype(BF16), v_s[h, pl.ds(j * CW, CW), :])
            sc = g_ref[pl.ds(r0, BQ), :] * (1.0 / jnp.sum(ml_s[1], axis=1, keepdims=True))
            return (c * jnp.concatenate([sc, sc], axis=1)).astype(BF16)

        def out(i, ctx):
            acc_ref[:, pl.ds(i * BQ, BQ)] += _dot_nt(wo_buf[h], ctx)

        acc_ref[:, pl.ds(S - BQ, BQ)] += _dot_nt(wo_buf[jnp.maximum(h - 1, 0)], ctx_s[...])
        c = None
        for i in range(NB):
            s = qk(i)
            if c is not None:
                out(i - 1, c)

                @pl.when(h == H - 1)
                def _():
                    ocopy(i - 1).start()
            c = pv(i, s)
        ctx_s[...] = c
        return carry

    ctx_s[...] = jnp.zeros((BQ, D), BF16)
    jax.lax.fori_loop(0, H, head, 0)
    acc_ref[:, pl.ds(S - BQ, BQ)] += _dot_nt(wo_buf[H - 1], ctx_s[...])
    ocopy(S // BQ - 1).start()
    for i in range(S // BQ):
        ocopy(i).wait()


BQ = 256
PRB = 1024
CW = 256


@jax.jit
def pallas_gated_mix__compressed_kv_cla__ssm_conv_s5__prompt_kernel(
      A_x, A_c_kv, A_w_q, A_w_uk, A_w_uv, A_w_o, B_x, B_Lambda_re, B_Lambda_im, B_B_re, B_B_im,
      B_C_re, B_C_im, B_log_dt, B_Dskip, gate_w):
    del B_x
    vm = pl.BlockSpec(memory_space=pltpu.VMEM)
    hbm = pl.BlockSpec(memory_space=pltpu.HBM)
    out = pl.pallas_call(
        _kernel,
        in_specs=[hbm] * 10 + [vm] * 5,
        out_specs=hbm,
        out_shape=jax.ShapeDtypeStruct((1, M, S), F32),
        scratch_shapes=[
            pltpu.VMEM((M, S), BF16),
            pltpu.VMEM((S, M), BF16),
            pltpu.VMEM((S, DC), BF16),
            pltpu.VMEM((2, M * 8, 128), U32),
            pltpu.VMEM((2, DC * 8, 128), U32),
            pltpu.VMEM((2, DC * 8, 128), U32),
            pltpu.VMEM((H, M, D), BF16),
            pltpu.VMEM((4, M, M), BF16),
            pltpu.SemaphoreType.DMA((16,)),
            pltpu.SemaphoreType.DMA((S // BQ,)),
            pltpu.VMEM((H, S, D), BF16),
            pltpu.VMEM((H, S, D), BF16),
            pltpu.VMEM((H, S, D), BF16),
            pltpu.VMEM((BQ, D), BF16),
            pltpu.VMEM((2, BQ, 128), F32),
            pltpu.VMEM((M, S), F32),
            pltpu.VMEM((S, 128), F32),
            pltpu.VMEM((4, NCH * PITCH, 128), F32),
            pltpu.VMEM((4, NCH * PITCH, 128), F32),
        ],
        compiler_params=pltpu.CompilerParams(vmem_limit_bytes=120 * 1024 * 1024),
    )(jnp.swapaxes(A_x, 1, 2), A_c_kv, A_w_q.reshape(M * H, D), A_w_uk.reshape(DC * H, D),
      A_w_uv.reshape(DC * H, D), jnp.swapaxes(A_w_o, 1, 2),
      B_B_re, B_B_im, B_C_re, B_C_im, B_Lambda_re, B_Lambda_im, B_log_dt, B_Dskip, gate_w)
    return jnp.swapaxes(out, 1, 2)
```

```python
import jax
import jax.numpy as jnp
import numpy as np
import jax.experimental.pallas as pl
import jax.experimental.pallas.tpu as pltpu

S = 2048
M = 448
H = 16
D = 256
DC = 1024
NCH = 8
TCH = S // NCH
PITCH = TCH + 4
LOG2E = 1.4426950408889634
NT = (((1,), (1,)), ((), ()))
F32 = jnp.float32
BF16 = jnp.bfloat16
U32 = jnp.uint32


def _dot(a, b):
    return jnp.dot(a, b, preferred_element_type=F32)


def _dot_nt(a, b):
    return jax.lax.dot_general(a, b, NT, preferred_element_type=F32)


def _cmul(ar, ai, br, bi):
    return ar * br - ai * bi, ar * bi + ai * br


def _a_sums(a11, a12, a21, a22):
    a11, a12, a21, a22 = (v.astype(F32) for v in (a11, a12, a21, a22))
    return [v.astype(BF16) for v in (a11 + a22, a21 + a22, a11 + a12, a21 - a11, a12 - a22)]


def _strassen(asum, a11, a22, b11, b12, b21, b22, put):
    m1 = _dot(asum(0), (b11 + b22).astype(BF16))
    m2 = _dot(asum(1), b11.astype(BF16))
    m4 = _dot(a22(), (b21 - b11).astype(BF16))
    put(1, 0, m2 + m4)
    u11 = m1 + m4
    m3 = _dot(a11(), (b12 - b22).astype(BF16))
    u22 = (m1 - m2) + m3
    m5 = _dot(asum(2), b22.astype(BF16))
    put(0, 1, m3 + m5)
    u11 = u11 - m5
    m6 = _dot(asum(3), (b11 + b12).astype(BF16))
    put(1, 1, u22 + m6)
    m7 = _dot(asum(4), (b21 + b22).astype(BF16))
    put(0, 0, u11 + m7)


def _lo16(v):
    return pltpu.bitcast(v << 16, F32)


def _hi16(v):
    return pltpu.bitcast(v & jnp.uint32(0xFFFF0000), F32)


def _tiles(v, sign):
    t = [v[:, j * 128:(j + 1) * 128] for j in range(3)]
    t.append(jnp.concatenate([v[:, 384:], sign * v[:, 384:]], axis=1))
    return t


def _ssm(xt_ref, x_ref, lre_ref, lim_ref, bre_ref, bim_ref, cre_ref, cim_ref, ldt_ref, dsk_ref, gw_ref,
         b_ref, g_ref, hre_ref, him_ref, pre_u, pre_y, pre_q, qproj, pre_2, csum, xs_ref):
    lre = lre_ref[...].astype(F32).reshape(1, M)
    lim = lim_ref[...].astype(F32).reshape(1, M)
    dt = jnp.exp(ldt_ref[...].astype(F32).reshape(1, M)).astype(BF16).astype(F32)
    mag = jnp.exp(dt * lre)
    ang = dt * lim
    ar = mag * jnp.cos(ang)
    ai = mag * jnp.sin(ang)
    den = lre * lre + lim * lim
    cr = _tiles(((ar - 1.0) * lre + ai * lim) / den, 1.0)
    ci = _tiles((ai * lre - (ar - 1.0) * lim) / den, -1.0)
    RB = 512
    pre_u(0)
    bre = bre_ref[...]
    bim = bim_ref[...]
    bcat = jnp.concatenate([bre[:384], bim[:384], bre[384:], bim[384:]], axis=0)
    for r in range(S // RB):
        rows = pl.ds(r * RB, RB)
        if r > 0:
            pre_u(r)
        xb = xt_ref[:, rows].T
        xp = jnp.concatenate([xb, jnp.zeros((RB, 512 - M), BF16)], axis=1)
        x_ref[rows, :] = xp
        if r >= 2:
            for o in range(0, RB, 16):
                lo = pl.ds((r - 2) * RB + o, 16)
                up = pl.ds(r * RB + o, 16)
                for j, v in enumerate(_a_sums(x_ref[lo, :256], x_ref[lo, 256:], x_ref[up, :256], x_ref[up, 256:])):
                    xs_ref[j, lo, :] = v
        u = _dot_nt(xb, bcat)
        for j in range(4):
            if j < 3:
                ur = u[:, j * 128:(j + 1) * 128]
                ui = u[:, 384 + j * 128:384 + (j + 1) * 128]
            else:
                ur = u[:, 768:]
                ui = pltpu.roll(ur, 64, 1)
            br, bi = _cmul(cr[j], ci[j], ur, ui)
            for cc in range(RB // TCH):
                dst = pl.ds((r * (RB // TCH) + cc) * PITCH, TCH)
                hre_ref[j, dst, :] = br[cc * TCH:(cc + 1) * TCH]
                him_ref[j, dst, :] = bi[cc * TCH:(cc + 1) * TCH]
    A_r = [jnp.broadcast_to(v, (NCH, 128)) for v in _tiles(ar, 1.0)]
    A_i = [jnp.broadcast_to(v, (NCH, 128)) for v in _tiles(ai, -1.0)]

    def mul_state(Ar, Ai, st):
        o = [_cmul(Ar[j], Ai[j], st[0][j], st[1][j]) for j in range(4)]
        return [a for a, _ in o], [b for _, b in o]

    def load(t):
        idx = pl.ds(t, NCH, stride=PITCH)
        return [hre_ref[j, idx, :] for j in range(4)], [him_ref[j, idx, :] for j in range(4)]

    def add(a, b):
        return [p + q for p, q in zip(a[0], b[0])], [p + q for p, q in zip(a[1], b[1])]

    def step1(t, st):
        return add(mul_state(A_r, A_i, st), load(t))

    z = jnp.zeros((NCH, 128), F32)
    NQ = H // 4
    SPI = TCH // NQ

    def loop1(p, st):
        qproj(p)
        for t in range(SPI):
            st = step1(p * SPI + t, st)
        return st

    pre_q()
    end = jax.lax.fori_loop(0, NQ, loop1, ([z] * 4, [z] * 4))
    Pr, Pi = A_r, A_i

    def square(Pr, Pi):
        return [a * a - b * b for a, b in zip(Pr, Pi)], [2.0 * a * b for a, b in zip(Pr, Pi)]

    for _ in range(int(np.log2(TCH))):
        Pr, Pi = square(Pr, Pi)
    row = jax.lax.broadcasted_iota(jnp.int32, (NCH, 128), 0)

    def shift(st, k):
        f = lambda v: jnp.where(row >= k, pltpu.roll(v, k, 0), 0.0)
        return [f(v) for v in st[0]], [f(v) for v in st[1]]

    car = shift(end, 1)
    k = 1
    while k < NCH:
        car = add(car, mul_state(Pr, Pi, shift(car, k)))
        Pr, Pi = square(Pr, Pi)
        k *= 2

    def step2(t, st):
        st = add(mul_state(A_r, A_i, st), load(t))
        idx = pl.ds(t, NCH, stride=PITCH)
        for j in range(4):
            hre_ref[j, idx, :] = st[0][j]
        for j in range(3):
            him_ref[j, idx, :] = st[1][j]
        return st

    def loop2(p, st):
        qproj(NQ + p)
        csum(p * 256, 256)
        for t in range(SPI):
            st = step2(p * SPI + t, st)
        return st

    pre_2()
    jax.lax.fori_loop(0, NQ, loop2, car)
    dsk = jnp.broadcast_to(dsk_ref[...].astype(F32).reshape(1, M), (128, M)).T
    gw = jnp.broadcast_to(gw_ref[...].astype(F32).reshape(1, M), (128, M)).T
    dsk = jnp.concatenate([dsk] * (RB // 128), axis=1)
    gw = jnp.concatenate([gw] * (RB // 128), axis=1)
    pre_y()
    cre = cre_ref[...]
    cim = cim_ref[...]
    ccat = jnp.concatenate([cre[:, :384], -cim[:, :384], cre[:, 384:], -cim[:, 384:]], axis=1)
    for r in range(S // RB):
        rows = pl.ds(r * RB, RB)
        def ld(ref, j):
            return jnp.concatenate([ref[j, pl.ds((r * (RB // TCH) + cc) * PITCH, TCH), :].astype(BF16)
                                    for cc in range(RB // TCH)], axis=0)
        hcat = jnp.concatenate([ld(hre_ref, j) for j in range(3)] + [ld(him_ref, j) for j in range(3)]
                               + [ld(hre_ref, 3)], axis=1)
        xf = xt_ref[:, rows].astype(F32)
        y = 2.0 * _dot_nt(ccat, hcat) + xf * dsk
        g = jax.nn.sigmoid(jnp.sum(xf * gw, axis=0, keepdims=True))
        b_ref[:, rows] = (1.0 - g) * y
        g_ref[rows, :] = jnp.broadcast_to(g, (128, RB)).T


def _kernel(xt_hbm, c_hbm, wq_hbm, wk_hbm, wv_hbm, wo_hbm, bre_hbm, bim_hbm, cre_hbm, cim_hbm,
            lre_ref, lim_ref, ldt_ref, dsk_ref, gw_ref,
            o_hbm,
            xt_ref, x_ref, c_ref, wq_buf, wk_buf, wv_buf, wo_buf, bc_buf, sems, osem,
            q_s, k_s, v_s, ctx_s, ml_s, cs_ref, xs_ref, acc_ref, g_ref, hre_ref, him_ref):
    def wcopies(w_hbm, buf, i):
        wu = w_hbm.bitcast(U32)
        return [pltpu.make_async_copy(wu.at[:, pl.ds(128 * j, 128)], buf.at[j], sems.at[i + j]) for j in range(2)]

    cp_x = [pltpu.make_async_copy(xt_hbm.at[0, :, pl.ds(512 * r, 512)], xt_ref.at[:, pl.ds(512 * r, 512)],
                                  sems.at[r]) for r in range(4)]
    cp_bc = [pltpu.make_async_copy(w, bc_buf.at[j], sems.at[4 + j])
             for j, w in enumerate((bre_hbm, bim_hbm, cre_hbm, cim_hbm))]
    cp_q = wcopies(wq_hbm, wq_buf, 8)
    rest = ([pltpu.make_async_copy(c_hbm.at[0], c_ref, sems.at[10])]
            + wcopies(wk_hbm, wk_buf, 11) + wcopies(wv_hbm, wv_buf, 13)
            + [pltpu.make_async_copy(wo_hbm, wo_buf, sems.at[15])])
    for cp in (cp_x[0], cp_bc[0], cp_bc[1]):
        cp.start()

    def pre_u(r):
        if r == 0:
            for cp in (cp_x[0], cp_bc[0], cp_bc[1]):
                cp.wait()
            for cp in cp_x[1:]:
                cp.start()
        else:
            cp_x[r].wait()
        if r == 1:
            for cp in cp_q:
                cp.start()

    def pre_q():
        for cp in cp_q:
            cp.wait()
        for cp in cp_bc[2:] + rest[:3]:
            cp.start()

    def pre_y():
        cp_bc[2].wait()
        cp_bc[3].wait()

    def pre_2():
        rest[0].wait()
        for cp in rest[3:]:
            cp.start()

    def csum(r0, n):
        HS, HK = S // 2, DC // 2
        for o in range(0, n, 16):
            lo = pl.ds(pl.multiple_of(r0 + o, 16), 16)
            up = pl.ds(pl.multiple_of(HS + r0 + o, 16), 16)
            for u in range(0, HK, 256):
                c0, c1 = pl.ds(u, 256), pl.ds(HK + u, 256)
                for j, v in enumerate(_a_sums(c_ref[lo, c0], c_ref[lo, c1], c_ref[up, c0], c_ref[up, c1])):
                    cs_ref[j, lo, c0] = v

    def qproj(p):
        HS = S // 2
        blocks = []
        for r0, n in ((0, 256), (256, M - 256)):
            for j in range(2):
                w = wq_buf[j, pl.ds(p + 8 * r0, n, stride=8), :]
                v = jnp.concatenate([_lo16(w), _hi16(w)], axis=1)
                if n < 256:
                    v = jnp.concatenate([v, jnp.zeros((256 - n, 256), F32)], axis=0)
                blocks.append(v)

        def put(r, c, v):
            v = (v * (LOG2E / 16.0)).astype(BF16)
            for e in range(2):
                q_s[2 * p + e, pl.ds(r * HS, HS), pl.ds(c * 128, 128)] = v[:, e * 128:(e + 1) * 128]

        _strassen(lambda j: xs_ref[j], lambda: x_ref[:HS, :256], lambda: x_ref[HS:, 256:], *blocks, put)

    _ssm(xt_ref, x_ref, lre_ref, lim_ref, bc_buf.at[0], bc_buf.at[1], bc_buf.at[2], bc_buf.at[3],
         ldt_ref, dsk_ref, gw_ref, acc_ref, g_ref, hre_ref, him_ref, pre_u, pre_y, pre_q, qproj, pre_2, csum, xs_ref)
    for cp in rest[1:]:
        cp.wait()

    def ocopy(i):
        cols = pl.ds(i * BQ, BQ)
        return pltpu.make_async_copy(acc_ref.at[:, cols], o_hbm.at[0, :, cols], osem.at[i])

    def kvproj(i, carry):
        HS, HK = S // 2, DC // 2
        for buf, dst in ((wk_buf, k_s), (wv_buf, v_s)):
            w = [buf[j, pl.ds(i + 8 * HK * r, HK, stride=8), :] for r in range(2) for j in range(2)]
            for e, f in enumerate((_lo16, _hi16)):
                def put(r, c, v, hh=2 * i + e, dst=dst):
                    dst[hh, pl.ds(r * HS, HS), pl.ds(c * 128, 128)] = v.astype(BF16)
                _strassen(lambda j: cs_ref[j], lambda: c_ref[:HS, :HK], lambda: c_ref[HS:, HK:],
                          *[f(v) for v in w], put)
        return carry

    jax.lax.fori_loop(0, H // 2, kvproj, 0)

    def head(h, carry):
        NB = S // BQ
        HB = BQ // 2

        def tri(n):
            ri = jax.lax.broadcasted_iota(jnp.int32, (n, n), 0)
            ci = jax.lax.broadcasted_iota(jnp.int32, (n, n), 1)
            return ci <= ri

        def qk(i):
            r0 = i * BQ
            q = q_s[h, pl.ds(r0, BQ), :]
            ss = [_dot_nt(q, k_s[h, pl.ds(j * CW, CW), :]) for j in range(r0 // CW)]
            sa = _dot_nt(q, k_s[h, pl.ds(r0, HB), :])
            sb = _dot_nt(q_s[h, pl.ds(r0 + HB, HB), :], k_s[h, pl.ds(r0 + HB, HB), :])
            t = tri(HB)
            sa = jnp.concatenate([jnp.where(t, sa[:HB], -1e9), sa[HB:]], axis=0)
            sb = jnp.where(t, sb, -1e9)
            mx = sa
            for sj in ss:
                for u in range(CW // 128):
                    mx = jnp.maximum(mx, sj[:, u * 128:(u + 1) * 128])
            mx = jnp.concatenate([mx[:HB], jnp.maximum(mx[HB:], sb)], axis=0)
            m = jnp.broadcast_to(jnp.max(mx, axis=1, keepdims=True), (BQ, 128))
            ml_s[0] = m
            return ss, sa, sb

        def pv(i, st):
            r0 = i * BQ
            ss, sa, sb = st
            m = ml_s[0]
            pa = jnp.exp2(sa - m)
            pb = jnp.exp2(sb - m[HB:])
            ml_s[1] = jnp.concatenate([pa[:HB], pa[HB:] + pb], axis=0)
            c = _dot(pa.astype(BF16), v_s[h, pl.ds(r0, HB), :])
            c = jnp.concatenate([c[:HB], c[HB:] + _dot(pb.astype(BF16), v_s[h, pl.ds(r0 + HB, HB), :])], axis=0)
            for j, sj in enumerate(ss):
                m = ml_s[0]
                ps = [jnp.exp2(sj[:, u * 128:(u + 1) * 128] - m) for u in range(CW // 128)]
                l = ml_s[1]
                for p in ps:
                    l = l + p
                ml_s[1] = l
                c = c + _dot(jnp.concatenate(ps, axis=1).astype(BF16), v_s[h, pl.ds(j * CW, CW), :])
            sc = g_ref[pl.ds(r0, BQ), :] * (1.0 / jnp.sum(ml_s[1], axis=1, keepdims=True))
            return (c * jnp.concatenate([sc, sc], axis=1)).astype(BF16)

        def out(i, ctx):
            acc_ref[:, pl.ds(i * BQ, BQ)] += _dot_nt(wo_buf[h], ctx)

        acc_ref[:, pl.ds(S - BQ, BQ)] += _dot_nt(wo_buf[jnp.maximum(h - 1, 0)], ctx_s[...])
        c = None
        for i in range(NB):
            s = qk(i)
            if c is not None:
                out(i - 1, c)

                @pl.when(h == H - 1)
                def _():
                    ocopy(i - 1).start()
            c = pv(i, s)
        ctx_s[...] = c
        return carry

    ctx_s[...] = jnp.zeros((BQ, D), BF16)
    jax.lax.fori_loop(0, H, head, 0)
    acc_ref[:, pl.ds(S - BQ, BQ)] += _dot_nt(wo_buf[H - 1], ctx_s[...])
    ocopy(S // BQ - 1).start()
    for i in range(S // BQ):
        ocopy(i).wait()


BQ = 256
CW = 256


@jax.jit
def pallas_gated_mix__compressed_kv_cla__ssm_conv_s5__prompt_kernel(
      A_x, A_c_kv, A_w_q, A_w_uk, A_w_uv, A_w_o, B_x, B_Lambda_re, B_Lambda_im, B_B_re, B_B_im,
      B_C_re, B_C_im, B_log_dt, B_Dskip, gate_w):
    del B_x
    vm = pl.BlockSpec(memory_space=pltpu.VMEM)
    hbm = pl.BlockSpec(memory_space=pltpu.HBM)
    out = pl.pallas_call(
        _kernel,
        in_specs=[hbm] * 10 + [vm] * 5,
        out_specs=hbm,
        out_shape=jax.ShapeDtypeStruct((1, M, S), F32),
        scratch_shapes=[
            pltpu.VMEM((M, S), BF16),
            pltpu.VMEM((S, 512), BF16),
            pltpu.VMEM((S, DC), BF16),
            pltpu.VMEM((2, M * 8, 128), U32),
            pltpu.VMEM((2, DC * 8, 128), U32),
            pltpu.VMEM((2, DC * 8, 128), U32),
            pltpu.VMEM((H, M, D), BF16),
            pltpu.VMEM((4, M, M), BF16),
            pltpu.SemaphoreType.DMA((16,)),
            pltpu.SemaphoreType.DMA((S // BQ,)),
            pltpu.VMEM((H, S, D), BF16),
            pltpu.VMEM((H, S, D), BF16),
            pltpu.VMEM((H, S, D), BF16),
            pltpu.VMEM((BQ, D), BF16),
            pltpu.VMEM((2, BQ, 128), F32),
            pltpu.VMEM((5, S // 2, DC // 2), BF16),
            pltpu.VMEM((5, S // 2, 256), BF16),
            pltpu.VMEM((M, S), F32),
            pltpu.VMEM((S, 128), F32),
            pltpu.VMEM((4, NCH * PITCH, 128), F32),
            pltpu.VMEM((4, NCH * PITCH, 128), F32),
        ],
        compiler_params=pltpu.CompilerParams(vmem_limit_bytes=120 * 1024 * 1024),
    )(jnp.swapaxes(A_x, 1, 2), A_c_kv, A_w_q.reshape(M * H, D), A_w_uk.reshape(DC * H, D),
      A_w_uv.reshape(DC * H, D), jnp.swapaxes(A_w_o, 1, 2),
      B_B_re, B_B_im, B_C_re, B_C_im, B_Lambda_re, B_Lambda_im, B_log_dt, B_Dskip, gate_w)
    return jnp.swapaxes(out, 1, 2)
```

```python
import functools

import jax
import jax.numpy as jnp
import numpy as np
import jax.experimental.pallas as pl
import jax.experimental.pallas.tpu as pltpu

S = 2048
M = 448
H = 16
D = 256
DC = 1024
NCH = 8
TCH = S // NCH
PITCH = TCH + 4
LOG2E = 1.4426950408889634
NT = (((1,), (1,)), ((), ()))
F32 = jnp.float32
BF16 = jnp.bfloat16
U32 = jnp.uint32


def _dot(a, b):
    return jnp.dot(a, b, preferred_element_type=F32)


def _dot_nt(a, b):
    return jax.lax.dot_general(a, b, NT, preferred_element_type=F32)


def _cmul(ar, ai, br, bi):
    return ar * br - ai * bi, ar * bi + ai * br


def _pow2(m):
    e = pltpu.bitcast(m, jnp.int32) & 0x7F800000
    e = jnp.minimum(jnp.maximum(e, 64 << 23), 190 << 23)
    return pltpu.bitcast(e, F32), pltpu.bitcast((254 << 23) - e, F32)


def _rep(v, n):
    return jnp.concatenate([v] * (n // 128), axis=1)


def _row_stats(a_ref, rs_ref, r0, n, cmax):
    for o in range(0, n, 16):
        rows = pl.ds(pl.multiple_of(r0 + o, 16), 16)
        t = [jnp.abs(a_ref[rows, pl.ds(j * 128, 128)].astype(F32)) for j in range(len(cmax))]
        m = functools.reduce(jnp.maximum, t)
        r, rinv = _pow2(jnp.broadcast_to(jnp.max(m, axis=1, keepdims=True), (16, 128)))
        rs_ref[rows, :] = r
        t = [v * rinv for v in t]
        cmax = [jnp.maximum(c, jnp.maximum(v[:8], v[8:])) for c, v in zip(cmax, t)]
    return cmax


def _col_scales(cmax, dk_ref):
    inv = []
    for j, c in enumerate(cmax):
        d, dinv = _pow2(jnp.broadcast_to(jnp.max(c, axis=0, keepdims=True), (8, 128)))
        dk_ref[pl.ds(j * 128, 128), :] = jnp.broadcast_to(d[:1], (128, 128)).T
        inv.append(jnp.concatenate([dinv, dinv], axis=0))
    return inv


def _a_operands(a_ref, rs_ref, dinv, dst_ref, r0, n):
    nk = len(dinv) // 2
    for o in range(r0, r0 + n, 16):
        lo, up = pl.ds(o, 16), pl.ds(S // 2 + o, 16)
        (rl, rli), (ru, rui) = _pow2(rs_ref[lo, :]), _pow2(rs_ref[up, :])
        sig = rl * rui
        rs_ref[up, :] = ru * rli
        for j in range(nk):
            c0, c1 = pl.ds(j * 128, 128), pl.ds((nk + j) * 128, 128)
            a11 = a_ref[lo, c0].astype(F32) * dinv[j]
            a12 = a_ref[lo, c1].astype(F32) * dinv[nk + j]
            a21 = a_ref[up, c0].astype(F32) * sig * dinv[j]
            a22 = a_ref[up, c1].astype(F32) * sig * dinv[nk + j]
            for i, v in enumerate((a11 + a22, a21 + a22, a11, a22, a11 + a12, a21 - a11, a12 - a22)):
                dst_ref[i, lo, c0] = v.astype(BF16)


def _strassen(a_ref, rs_ref, dk_ref, b11, b12, b21, b22, put):
    kh, nh = b11.shape
    d1, d2 = _rep(dk_ref[pl.ds(0, kh), :], nh), _rep(dk_ref[pl.ds(kh, kh), :], nh)
    b11, b12, b21, b22 = b11 * d1, b12 * d1, b21 * d2, b22 * d2

    def colscale(top, bot):
        m = jnp.max(jnp.maximum(jnp.abs(top), jnp.abs(bot)), axis=0, keepdims=True)
        return _pow2(jnp.broadcast_to(m, (8, nh)))

    (c1, c1i), (c2, c2i) = colscale(b11, b21), colscale(b12, b22)
    rho, rhoi = (c1 * c2i)[:1], (c2 * c1i)[:1]
    unrow = lambda v: v * _rep(rs_ref[pl.ds(S // 2, S // 2), :], nh)

    m2 = _dot(a_ref[1], b11.astype(BF16))
    m4 = _dot(a_ref[3], (b21 - b11).astype(BF16))
    put(1, 0, unrow(m2 + m4))
    m3 = _dot(a_ref[2], (b12 - b22).astype(BF16))
    m5 = _dot(a_ref[4], b22.astype(BF16))
    put(0, 1, m3 + m5)
    u11 = m4 - m5 * rho
    b22 = b22 * rho
    m1 = _dot(a_ref[0], (b11 + b22).astype(BF16))
    u11 = u11 + m1
    u22 = m1 - m2
    m6 = _dot(a_ref[5], (b11 + b12 * rho).astype(BF16))
    put(1, 1, unrow((u22 + m6) * rhoi + m3))
    m7 = _dot(a_ref[6], (b21 + b22).astype(BF16))
    put(0, 0, u11 + m7)


def _lo16(v):
    return pltpu.bitcast(v << 16, F32)


def _hi16(v):
    return pltpu.bitcast(v & jnp.uint32(0xFFFF0000), F32)


def _tiles(v, sign):
    t = [v[:, j * 128:(j + 1) * 128] for j in range(3)]
    t.append(jnp.concatenate([v[:, 384:], sign * v[:, 384:]], axis=1))
    return t


def _ssm(xt_ref, x_ref, lre_ref, lim_ref, bre_ref, bim_ref, cre_ref, cim_ref, ldt_ref, dsk_ref, gw_ref,
         b_ref, g_ref, hre_ref, him_ref, pre_u, pre_y, pre_q, qproj, pre_2, c_ref, rx, rc):
    xs_ref, rsx_ref, dx_ref = rx
    cs_ref, rsc_ref, dc_ref = rc
    lre = lre_ref[...].astype(F32).reshape(1, M)
    lim = lim_ref[...].astype(F32).reshape(1, M)
    dt = jnp.exp(ldt_ref[...].astype(F32).reshape(1, M)).astype(BF16).astype(F32)
    mag = jnp.exp(dt * lre)
    ang = dt * lim
    ar = mag * jnp.cos(ang)
    ai = mag * jnp.sin(ang)
    den = lre * lre + lim * lim
    cr = _tiles(((ar - 1.0) * lre + ai * lim) / den, 1.0)
    ci = _tiles((ai * lre - (ar - 1.0) * lim) / den, -1.0)
    RB = 512
    pre_u(0)
    bre = bre_ref[...]
    bim = bim_ref[...]
    bcat = jnp.concatenate([bre[:384], bim[:384], bre[384:], bim[384:]], axis=0)
    z = jnp.zeros((8, 128), F32)
    xmax = [z] * 4
    for r in range(S // RB):
        rows = pl.ds(r * RB, RB)
        if r > 0:
            pre_u(r)
        xb = xt_ref[:, rows].T
        xp = jnp.concatenate([xb, jnp.zeros((RB, 512 - M), BF16)], axis=1)
        x_ref[rows, :] = xp
        xmax = _row_stats(x_ref, rsx_ref, r * RB, RB, xmax)
        if r == S // RB - 1:
            _a_operands(x_ref, rsx_ref, _col_scales(xmax, dx_ref), xs_ref, 0, S // 2)
        u = _dot_nt(xb, bcat)
        for j in range(4):
            if j < 3:
                ur = u[:, j * 128:(j + 1) * 128]
                ui = u[:, 384 + j * 128:384 + (j + 1) * 128]
            else:
                ur = u[:, 768:]
                ui = pltpu.roll(ur, 64, 1)
            br, bi = _cmul(cr[j], ci[j], ur, ui)
            for cc in range(RB // TCH):
                dst = pl.ds((r * (RB // TCH) + cc) * PITCH, TCH)
                hre_ref[j, dst, :] = br[cc * TCH:(cc + 1) * TCH]
                him_ref[j, dst, :] = bi[cc * TCH:(cc + 1) * TCH]
    A_r = [jnp.broadcast_to(v, (NCH, 128)) for v in _tiles(ar, 1.0)]
    A_i = [jnp.broadcast_to(v, (NCH, 128)) for v in _tiles(ai, -1.0)]

    def mul_state(Ar, Ai, st):
        o = [_cmul(Ar[j], Ai[j], st[0][j], st[1][j]) for j in range(4)]
        return [a for a, _ in o], [b for _, b in o]

    def load(t):
        idx = pl.ds(t, NCH, stride=PITCH)
        return [hre_ref[j, idx, :] for j in range(4)], [him_ref[j, idx, :] for j in range(4)]

    def add(a, b):
        return [p + q for p, q in zip(a[0], b[0])], [p + q for p, q in zip(a[1], b[1])]

    def step1(t, st):
        return add(mul_state(A_r, A_i, st), load(t))

    z = jnp.zeros((NCH, 128), F32)
    NQ = H // 4
    SPI = TCH // NQ

    def loop1(p, st):
        qproj(p)
        for t in range(SPI):
            st = step1(p * SPI + t, st)
        return st

    pre_q()
    end = jax.lax.fori_loop(0, NQ, loop1, ([z] * 4, [z] * 4))
    Pr, Pi = A_r, A_i

    def square(Pr, Pi):
        return [a * a - b * b for a, b in zip(Pr, Pi)], [2.0 * a * b for a, b in zip(Pr, Pi)]

    for _ in range(int(np.log2(TCH))):
        Pr, Pi = square(Pr, Pi)
    row = jax.lax.broadcasted_iota(jnp.int32, (NCH, 128), 0)

    def shift(st, k):
        f = lambda v: jnp.where(row >= k, pltpu.roll(v, k, 0), 0.0)
        return [f(v) for v in st[0]], [f(v) for v in st[1]]

    car = shift(end, 1)
    k = 1
    while k < NCH:
        car = add(car, mul_state(Pr, Pi, shift(car, k)))
        Pr, Pi = square(Pr, Pi)
        k *= 2

    def step2(t, st):
        st = add(mul_state(A_r, A_i, st), load(t))
        idx = pl.ds(t, NCH, stride=PITCH)
        for j in range(4):
            hre_ref[j, idx, :] = st[0][j]
        for j in range(3):
            him_ref[j, idx, :] = st[1][j]
        return st

    def loop2(p, carry):
        st, cmax = carry
        qproj(NQ + p)
        cmax = _row_stats(c_ref, rsc_ref, p * (S // NQ), S // NQ, cmax)
        for t in range(SPI):
            st = step2(p * SPI + t, st)
        return st, cmax

    pre_2()
    _, cmax = jax.lax.fori_loop(0, NQ, loop2, (car, [z] * (DC // 128)))
    dcinv = _col_scales(cmax, dc_ref)
    dsk = jnp.broadcast_to(dsk_ref[...].astype(F32).reshape(1, M), (128, M)).T
    gw = jnp.broadcast_to(gw_ref[...].astype(F32).reshape(1, M), (128, M)).T
    dsk = jnp.concatenate([dsk] * (RB // 128), axis=1)
    gw = jnp.concatenate([gw] * (RB // 128), axis=1)
    pre_y()
    cre = cre_ref[...]
    cim = cim_ref[...]
    ccat = jnp.concatenate([cre[:, :384], -cim[:, :384], cre[:, 384:], -cim[:, 384:]], axis=1)
    for r in range(S // RB):
        rows = pl.ds(r * RB, RB)
        def ld(ref, j):
            return jnp.concatenate([ref[j, pl.ds((r * (RB // TCH) + cc) * PITCH, TCH), :].astype(BF16)
                                    for cc in range(RB // TCH)], axis=0)
        hcat = jnp.concatenate([ld(hre_ref, j) for j in range(3)] + [ld(him_ref, j) for j in range(3)]
                               + [ld(hre_ref, 3)], axis=1)
        xf = xt_ref[:, rows].astype(F32)
        y = 2.0 * _dot_nt(ccat, hcat) + xf * dsk
        g = jax.nn.sigmoid(jnp.sum(xf * gw, axis=0, keepdims=True))
        b_ref[:, rows] = (1.0 - g) * y
        _a_operands(c_ref, rsc_ref, dcinv, cs_ref, r * (RB // 2), RB // 2)
        g_ref[rows, :] = jnp.broadcast_to(g, (128, RB)).T


def _kernel(xt_hbm, c_hbm, wq_hbm, wk_hbm, wv_hbm, wo_hbm, bre_hbm, bim_hbm, cre_hbm, cim_hbm,
            lre_ref, lim_ref, ldt_ref, dsk_ref, gw_ref,
            o_hbm,
            xt_ref, x_ref, c_ref, wq_buf, wk_buf, wv_buf, wo_buf, bc_buf, sems, osem,
            q_s, k_s, v_s, ctx_s, ml_s, cs_ref, xs_ref, rsc_ref, rsx_ref, dc_ref, dx_ref,
            acc_ref, g_ref, hre_ref, him_ref):
    def wcopies(w_hbm, buf, i):
        wu = w_hbm.bitcast(U32)
        return [pltpu.make_async_copy(wu.at[:, pl.ds(128 * j, 128)], buf.at[j], sems.at[i + j]) for j in range(2)]

    cp_x = [pltpu.make_async_copy(xt_hbm.at[0, :, pl.ds(512 * r, 512)], xt_ref.at[:, pl.ds(512 * r, 512)],
                                  sems.at[r]) for r in range(4)]
    cp_bc = [pltpu.make_async_copy(w, bc_buf.at[j], sems.at[4 + j])
             for j, w in enumerate((bre_hbm, bim_hbm, cre_hbm, cim_hbm))]
    cp_q = wcopies(wq_hbm, wq_buf, 8)
    rest = ([pltpu.make_async_copy(c_hbm.at[0], c_ref, sems.at[10])]
            + wcopies(wk_hbm, wk_buf, 11) + wcopies(wv_hbm, wv_buf, 13)
            + [pltpu.make_async_copy(wo_hbm, wo_buf, sems.at[15])])
    for cp in (cp_x[0], cp_bc[0], cp_bc[1]):
        cp.start()

    def pre_u(r):
        if r == 0:
            for cp in (cp_x[0], cp_bc[0], cp_bc[1]):
                cp.wait()
            for cp in cp_x[1:]:
                cp.start()
        else:
            cp_x[r].wait()
        if r == 1:
            for cp in cp_q:
                cp.start()

    def pre_q():
        for cp in cp_q:
            cp.wait()
        for cp in cp_bc[2:] + rest[:3]:
            cp.start()

    def pre_y():
        cp_bc[2].wait()
        cp_bc[3].wait()

    def pre_2():
        rest[0].wait()
        for cp in rest[3:]:
            cp.start()

    def qproj(p):
        HS = S // 2
        blocks = []
        for r0, n in ((0, 256), (256, M - 256)):
            for j in range(2):
                w = wq_buf[j, pl.ds(p + 8 * r0, n, stride=8), :]
                v = jnp.concatenate([_lo16(w), _hi16(w)], axis=1)
                if n < 256:
                    v = jnp.concatenate([v, jnp.zeros((256 - n, 256), F32)], axis=0)
                blocks.append(v)

        def put(r, c, v):
            v = (v * (LOG2E / 16.0)).astype(BF16)
            for e in range(2):
                q_s[2 * p + e, pl.ds(r * HS, HS), pl.ds(c * 128, 128)] = v[:, e * 128:(e + 1) * 128]

        _strassen(xs_ref, rsx_ref, dx_ref, *blocks, put)

    _ssm(xt_ref, x_ref, lre_ref, lim_ref, bc_buf.at[0], bc_buf.at[1], bc_buf.at[2], bc_buf.at[3],
         ldt_ref, dsk_ref, gw_ref, acc_ref, g_ref, hre_ref, him_ref, pre_u, pre_y, pre_q, qproj, pre_2,
         c_ref, (xs_ref, rsx_ref, dx_ref), (cs_ref, rsc_ref, dc_ref))
    for cp in rest[1:]:
        cp.wait()

    def ocopy(i):
        cols = pl.ds(i * BQ, BQ)
        return pltpu.make_async_copy(acc_ref.at[:, cols], o_hbm.at[0, :, cols], osem.at[i])

    def kvproj(i, carry):
        HS, HK = S // 2, DC // 2
        for buf, dst in ((wk_buf, k_s), (wv_buf, v_s)):
            w = [buf[j, pl.ds(i + 8 * HK * r, HK, stride=8), :] for r in range(2) for j in range(2)]
            for e, f in enumerate((_lo16, _hi16)):
                def put(r, c, v, hh=2 * i + e, dst=dst):
                    dst[hh, pl.ds(r * HS, HS), pl.ds(c * 128, 128)] = v.astype(BF16)
                _strassen(cs_ref, rsc_ref, dc_ref, *[f(v) for v in w], put)
        return carry

    jax.lax.fori_loop(0, H // 2, kvproj, 0)

    def head(h, carry):
        NB = S // BQ
        HB = BQ // 2

        def tri(n):
            ri = jax.lax.broadcasted_iota(jnp.int32, (n, n), 0)
            ci = jax.lax.broadcasted_iota(jnp.int32, (n, n), 1)
            return ci <= ri

        def qk(i):
            r0 = i * BQ
            q = q_s[h, pl.ds(r0, BQ), :]
            ss = [_dot_nt(q, k_s[h, pl.ds(j * CW, CW), :]) for j in range(r0 // CW)]
            sa = _dot_nt(q, k_s[h, pl.ds(r0, HB), :])
            sb = _dot_nt(q_s[h, pl.ds(r0 + HB, HB), :], k_s[h, pl.ds(r0 + HB, HB), :])
            t = tri(HB)
            sa = jnp.concatenate([jnp.where(t, sa[:HB], -1e9), sa[HB:]], axis=0)
            sb = jnp.where(t, sb, -1e9)
            mx = sa
            for sj in ss:
                for u in range(CW // 128):
                    mx = jnp.maximum(mx, sj[:, u * 128:(u + 1) * 128])
            mx = jnp.concatenate([mx[:HB], jnp.maximum(mx[HB:], sb)], axis=0)
            m = jnp.broadcast_to(jnp.max(mx, axis=1, keepdims=True), (BQ, 128))
            ml_s[0] = m
            return ss, sa, sb

        def pv(i, st):
            r0 = i * BQ
            ss, sa, sb = st
            m = ml_s[0]
            pa = jnp.exp2(sa - m)
            pb = jnp.exp2(sb - m[HB:])
            ml_s[1] = jnp.concatenate([pa[:HB], pa[HB:] + pb], axis=0)
            c = _dot(pa.astype(BF16), v_s[h, pl.ds(r0, HB), :])
            c = jnp.concatenate([c[:HB], c[HB:] + _dot(pb.astype(BF16), v_s[h, pl.ds(r0 + HB, HB), :])], axis=0)
            for j, sj in enumerate(ss):
                m = ml_s[0]
                ps = [jnp.exp2(sj[:, u * 128:(u + 1) * 128] - m) for u in range(CW // 128)]
                l = ml_s[1]
                for p in ps:
                    l = l + p
                ml_s[1] = l
                c = c + _dot(jnp.concatenate(ps, axis=1).astype(BF16), v_s[h, pl.ds(j * CW, CW), :])
            sc = g_ref[pl.ds(r0, BQ), :] * (1.0 / jnp.sum(ml_s[1], axis=1, keepdims=True))
            return (c * jnp.concatenate([sc, sc], axis=1)).astype(BF16)

        def out(i, ctx):
            acc_ref[:, pl.ds(i * BQ, BQ)] += _dot_nt(wo_buf[h], ctx)

        acc_ref[:, pl.ds(S - BQ, BQ)] += _dot_nt(wo_buf[jnp.maximum(h - 1, 0)], ctx_s[...])
        c = None
        for i in range(NB):
            s = qk(i)
            if c is not None:
                out(i - 1, c)

                @pl.when(h == H - 1)
                def _():
                    ocopy(i - 1).start()
            c = pv(i, s)
        ctx_s[...] = c
        return carry

    ctx_s[...] = jnp.zeros((BQ, D), BF16)
    jax.lax.fori_loop(0, H, head, 0)
    acc_ref[:, pl.ds(S - BQ, BQ)] += _dot_nt(wo_buf[H - 1], ctx_s[...])
    ocopy(S // BQ - 1).start()
    for i in range(S // BQ):
        ocopy(i).wait()


BQ = 256
CW = 256


@jax.jit
def pallas_gated_mix__compressed_kv_cla__ssm_conv_s5__prompt_kernel(
      A_x, A_c_kv, A_w_q, A_w_uk, A_w_uv, A_w_o, B_x, B_Lambda_re, B_Lambda_im, B_B_re, B_B_im,
      B_C_re, B_C_im, B_log_dt, B_Dskip, gate_w):
    del B_x
    vm = pl.BlockSpec(memory_space=pltpu.VMEM)
    hbm = pl.BlockSpec(memory_space=pltpu.HBM)
    out = pl.pallas_call(
        _kernel,
        in_specs=[hbm] * 10 + [vm] * 5,
        out_specs=hbm,
        out_shape=jax.ShapeDtypeStruct((1, M, S), F32),
        scratch_shapes=[
            pltpu.VMEM((M, S), BF16),
            pltpu.VMEM((S, 512), BF16),
            pltpu.VMEM((S, DC), BF16),
            pltpu.VMEM((2, M * 8, 128), U32),
            pltpu.VMEM((2, DC * 8, 128), U32),
            pltpu.VMEM((2, DC * 8, 128), U32),
            pltpu.VMEM((H, M, D), BF16),
            pltpu.VMEM((4, M, M), BF16),
            pltpu.SemaphoreType.DMA((16,)),
            pltpu.SemaphoreType.DMA((S // BQ,)),
            pltpu.VMEM((H, S, D), BF16),
            pltpu.VMEM((H, S, D), BF16),
            pltpu.VMEM((H, S, D), BF16),
            pltpu.VMEM((BQ, D), BF16),
            pltpu.VMEM((2, BQ, 128), F32),
            pltpu.VMEM((7, S // 2, DC // 2), BF16),
            pltpu.VMEM((7, S // 2, 256), BF16),
            pltpu.VMEM((S, 128), F32),
            pltpu.VMEM((S, 128), F32),
            pltpu.VMEM((DC, 128), F32),
            pltpu.VMEM((512, 128), F32),
            pltpu.VMEM((M, S), F32),
            pltpu.VMEM((S, 128), F32),
            pltpu.VMEM((4, NCH * PITCH, 128), F32),
            pltpu.VMEM((4, NCH * PITCH, 128), F32),
        ],
        compiler_params=pltpu.CompilerParams(vmem_limit_bytes=124 * 1024 * 1024),
    )(jnp.swapaxes(A_x, 1, 2), A_c_kv, A_w_q.reshape(M * H, D), A_w_uk.reshape(DC * H, D),
      A_w_uv.reshape(DC * H, D), jnp.swapaxes(A_w_o, 1, 2),
      B_B_re, B_B_im, B_C_re, B_C_im, B_Lambda_re, B_Lambda_im, B_log_dt, B_Dskip, gate_w)
    return jnp.swapaxes(out, 1, 2)
```

```python
import functools

import jax
import jax.numpy as jnp
import numpy as np
import jax.experimental.pallas as pl
import jax.experimental.pallas.tpu as pltpu

S = 2048
M = 448
H = 16
D = 256
DC = 1024
NCH = 8
TCH = S // NCH
PITCH = TCH + 4
LOG2E = 1.4426950408889634
NT = (((1,), (1,)), ((), ()))
F32 = jnp.float32
BF16 = jnp.bfloat16
U32 = jnp.uint32


def _dot(a, b):
    return jnp.dot(a, b, preferred_element_type=F32)


def _dot_nt(a, b):
    return jax.lax.dot_general(a, b, NT, preferred_element_type=F32)


def _cmul(ar, ai, br, bi):
    return ar * br - ai * bi, ar * bi + ai * br


def _pow2(m):
    e = pltpu.bitcast(m, jnp.int32) & 0x7F800000
    e = jnp.minimum(jnp.maximum(e, 64 << 23), 190 << 23)
    return pltpu.bitcast(e, F32), pltpu.bitcast((254 << 23) - e, F32)


def _rep(v, n):
    return jnp.concatenate([v] * (n // 128), axis=1)


def _row_stats(a_ref, rs_ref, r0, n, cmax):
    for o in range(0, n, 16):
        rows = pl.ds(pl.multiple_of(r0 + o, 16), 16)
        t = [jnp.abs(a_ref[rows, pl.ds(j * 128, 128)].astype(F32)) for j in range(len(cmax))]
        m = functools.reduce(jnp.maximum, t)
        r, rinv = _pow2(jnp.broadcast_to(jnp.max(m, axis=1, keepdims=True), (16, 128)))
        rs_ref[rows, :] = r
        t = [v * rinv for v in t]
        cmax = [jnp.maximum(c, jnp.maximum(v[:8], v[8:])) for c, v in zip(cmax, t)]
    return cmax


def _col_scales(cmax, dk_ref):
    inv = []
    for j, c in enumerate(cmax):
        d, dinv = _pow2(jnp.broadcast_to(jnp.max(c, axis=0, keepdims=True), (8, 128)))
        dk_ref[pl.ds(j * 128, 128), :] = jnp.broadcast_to(d[:1], (128, 128)).T
        inv.append(jnp.concatenate([dinv, dinv], axis=0))
    return inv


def _a_operands(a_ref, rs_ref, dinv, dst_ref, r0, n):
    nk = len(dinv) // 2
    for o in range(r0, r0 + n, 16):
        lo, up = pl.ds(o, 16), pl.ds(S // 2 + o, 16)
        (rl, rli), (ru, rui) = _pow2(rs_ref[lo, :]), _pow2(rs_ref[up, :])
        sig = rl * rui
        rs_ref[up, :] = ru * rli
        for j in range(nk):
            c0, c1 = pl.ds(j * 128, 128), pl.ds((nk + j) * 128, 128)
            a11 = a_ref[lo, c0].astype(F32) * dinv[j]
            a12 = a_ref[lo, c1].astype(F32) * dinv[nk + j]
            a21 = a_ref[up, c0].astype(F32) * sig * dinv[j]
            a22 = a_ref[up, c1].astype(F32) * sig * dinv[nk + j]
            for i, v in enumerate((a11 + a22, a21 + a22, a11, a22, a11 + a12, a21 - a11, a12 - a22)):
                dst_ref[i, lo, c0] = v.astype(BF16)


def _strassen(a_ref, rs_ref, dk_ref, b11, b12, b21, b22, put):
    kh, nh = b11.shape
    d1, d2 = _rep(dk_ref[pl.ds(0, kh), :], nh), _rep(dk_ref[pl.ds(kh, kh), :], nh)
    b11, b12, b21, b22 = b11 * d1, b12 * d1, b21 * d2, b22 * d2

    def colscale(top, bot):
        m = jnp.max(jnp.maximum(jnp.abs(top), jnp.abs(bot)), axis=0, keepdims=True)
        return _pow2(jnp.broadcast_to(m, (8, nh)))

    (c1, c1i), (c2, c2i) = colscale(b11, b21), colscale(b12, b22)
    rho, rhoi = (c1 * c2i)[:1], (c2 * c1i)[:1]
    unrow = lambda v: v * _rep(rs_ref[pl.ds(S // 2, S // 2), :], nh)

    m2 = _dot(a_ref[1], b11.astype(BF16))
    m4 = _dot(a_ref[3], (b21 - b11).astype(BF16))
    put(1, 0, unrow(m2 + m4))
    m3 = _dot(a_ref[2], (b12 - b22).astype(BF16))
    m5 = _dot(a_ref[4], b22.astype(BF16))
    put(0, 1, m3 + m5)
    u11 = m4 - m5 * rho
    b22 = b22 * rho
    m1 = _dot(a_ref[0], (b11 + b22).astype(BF16))
    u11 = u11 + m1
    u22 = m1 - m2
    m6 = _dot(a_ref[5], (b11 + b12 * rho).astype(BF16))
    put(1, 1, unrow((u22 + m6) * rhoi + m3))
    m7 = _dot(a_ref[6], (b21 + b22).astype(BF16))
    put(0, 0, u11 + m7)


def _lo16(v):
    return pltpu.bitcast(v << 16, F32)


def _hi16(v):
    return pltpu.bitcast(v & jnp.uint32(0xFFFF0000), F32)


def _tiles(v, sign):
    t = [v[:, j * 128:(j + 1) * 128] for j in range(3)]
    t.append(jnp.concatenate([v[:, 384:], sign * v[:, 384:]], axis=1))
    return t


def _ssm(xt_ref, x_ref, lre_ref, lim_ref, bre_ref, bim_ref, cre_ref, cim_ref, ldt_ref, dsk_ref, gw_ref,
         b_ref, g_ref, hre_ref, him_ref, pre_u, pre_y, pre_q, qproj, pre_2, c_ref, rx, rc):
    xs_ref, rsx_ref, dx_ref = rx
    cs_ref, rsc_ref, dc_ref = rc
    lre = lre_ref[...].astype(F32).reshape(1, M)
    lim = lim_ref[...].astype(F32).reshape(1, M)
    dt = jnp.exp(ldt_ref[...].astype(F32).reshape(1, M)).astype(BF16).astype(F32)
    mag = jnp.exp(dt * lre)
    ang = dt * lim
    ar = mag * jnp.cos(ang)
    ai = mag * jnp.sin(ang)
    den = lre * lre + lim * lim
    cr = _tiles(((ar - 1.0) * lre + ai * lim) / den, 1.0)
    ci = _tiles((ai * lre - (ar - 1.0) * lim) / den, -1.0)
    RB = 512
    pre_u(0)
    bre = bre_ref[...]
    bim = bim_ref[...]
    bcat = jnp.concatenate([bre[:384], bim[:384], bre[384:], bim[384:]], axis=0)
    z = jnp.zeros((8, 128), F32)
    xmax = [z] * 4
    for r in range(S // RB):
        rows = pl.ds(r * RB, RB)
        if r > 0:
            pre_u(r)
        xb = xt_ref[:, rows].T
        xp = jnp.concatenate([xb, jnp.zeros((RB, 512 - M), BF16)], axis=1)
        x_ref[rows, :] = xp
        xmax = _row_stats(x_ref, rsx_ref, r * RB, RB, xmax)
        if r == S // RB - 1:
            _a_operands(x_ref, rsx_ref, _col_scales(xmax, dx_ref), xs_ref, 0, S // 2)
        u = _dot_nt(xb, bcat)
        for j in range(4):
            if j < 3:
                ur = u[:, j * 128:(j + 1) * 128]
                ui = u[:, 384 + j * 128:384 + (j + 1) * 128]
            else:
                ur = u[:, 768:]
                ui = pltpu.roll(ur, 64, 1)
            br, bi = _cmul(cr[j], ci[j], ur, ui)
            for cc in range(RB // TCH):
                dst = pl.ds((r * (RB // TCH) + cc) * PITCH, TCH)
                hre_ref[j, dst, :] = br[cc * TCH:(cc + 1) * TCH]
                him_ref[j, dst, :] = bi[cc * TCH:(cc + 1) * TCH]
    A_r = [jnp.broadcast_to(v, (NCH, 128)) for v in _tiles(ar, 1.0)]
    A_i = [jnp.broadcast_to(v, (NCH, 128)) for v in _tiles(ai, -1.0)]

    def mul_state(Ar, Ai, st):
        o = [_cmul(Ar[j], Ai[j], st[0][j], st[1][j]) for j in range(4)]
        return [a for a, _ in o], [b for _, b in o]

    def load(t):
        idx = pl.ds(t, NCH, stride=PITCH)
        return [hre_ref[j, idx, :] for j in range(4)], [him_ref[j, idx, :] for j in range(4)]

    def add(a, b):
        return [p + q for p, q in zip(a[0], b[0])], [p + q for p, q in zip(a[1], b[1])]

    def step1(t, st):
        return add(mul_state(A_r, A_i, st), load(t))

    z = jnp.zeros((NCH, 128), F32)
    NQ = H // 4
    SPI = TCH // NQ

    def loop1(p, st):
        qproj(p)
        for t in range(SPI):
            st = step1(p * SPI + t, st)
        return st

    pre_q()
    end = jax.lax.fori_loop(0, NQ, loop1, ([z] * 4, [z] * 4))
    Pr, Pi = A_r, A_i

    def square(Pr, Pi):
        return [a * a - b * b for a, b in zip(Pr, Pi)], [2.0 * a * b for a, b in zip(Pr, Pi)]

    for _ in range(int(np.log2(TCH))):
        Pr, Pi = square(Pr, Pi)
    row = jax.lax.broadcasted_iota(jnp.int32, (NCH, 128), 0)

    def shift(st, k):
        f = lambda v: jnp.where(row >= k, pltpu.roll(v, k, 0), 0.0)
        return [f(v) for v in st[0]], [f(v) for v in st[1]]

    car = shift(end, 1)
    k = 1
    while k < NCH:
        car = add(car, mul_state(Pr, Pi, shift(car, k)))
        Pr, Pi = square(Pr, Pi)
        k *= 2

    def step2(t, st):
        st = add(mul_state(A_r, A_i, st), load(t))
        idx = pl.ds(t, NCH, stride=PITCH)
        for j in range(4):
            hre_ref[j, idx, :] = st[0][j]
        for j in range(3):
            him_ref[j, idx, :] = st[1][j]
        return st

    def loop2(p, carry):
        st, cmax = carry
        qproj(NQ + p)
        cmax = _row_stats(c_ref, rsc_ref, p * (S // NQ), S // NQ, cmax)
        for t in range(SPI):
            st = step2(p * SPI + t, st)
        return st, cmax

    pre_2()
    _, cmax = jax.lax.fori_loop(0, NQ, loop2, (car, [z] * (DC // 128)))
    dcinv = _col_scales(cmax, dc_ref)
    dsk = jnp.broadcast_to(dsk_ref[...].astype(F32).reshape(1, M), (128, M)).T
    gw = jnp.broadcast_to(gw_ref[...].astype(F32).reshape(1, M), (128, M)).T
    dsk = jnp.concatenate([dsk] * (RB // 128), axis=1)
    gw = jnp.concatenate([gw] * (RB // 128), axis=1)
    pre_y()
    cre = cre_ref[...]
    cim = cim_ref[...]
    ccat = jnp.concatenate([cre[:, :384], -cim[:, :384], cre[:, 384:], -cim[:, 384:]], axis=1)
    for r in range(S // RB):
        rows = pl.ds(r * RB, RB)
        def ld(ref, j):
            return jnp.concatenate([ref[j, pl.ds((r * (RB // TCH) + cc) * PITCH, TCH), :].astype(BF16)
                                    for cc in range(RB // TCH)], axis=0)
        hcat = jnp.concatenate([ld(hre_ref, j) for j in range(3)] + [ld(him_ref, j) for j in range(3)]
                               + [ld(hre_ref, 3)], axis=1)
        xf = xt_ref[:, rows].astype(F32)
        y = 2.0 * _dot_nt(ccat, hcat) + xf * dsk
        g = jax.nn.sigmoid(jnp.sum(xf * gw, axis=0, keepdims=True))
        b_ref[:, rows] = (1.0 - g) * y
        _a_operands(c_ref, rsc_ref, dcinv, cs_ref, r * (RB // 2), RB // 2)
        g_ref[rows, :] = jnp.broadcast_to(g, (128, RB)).T


def _kernel(xt_hbm, c_hbm, wq_hbm, wk_hbm, wv_hbm, wo_hbm, bre_hbm, bim_hbm, cre_hbm, cim_hbm,
            lre_ref, lim_ref, ldt_ref, dsk_ref, gw_ref,
            o_hbm,
            xt_ref, x_ref, c_ref, wq_buf, wk_buf, wv_buf, wo_buf, bc_buf, sems, osem,
            q_s, k_s, v_s, ctx_s, cs_ref, xs_ref, rsc_ref, rsx_ref, dc_ref, dx_ref,
            acc_ref, g_ref, hre_ref, him_ref):
    def wcopies(w_hbm, buf, i):
        wu = w_hbm.bitcast(U32)
        return [pltpu.make_async_copy(wu.at[:, pl.ds(128 * j, 128)], buf.at[j], sems.at[i + j]) for j in range(2)]

    cp_x = [pltpu.make_async_copy(xt_hbm.at[0, :, pl.ds(512 * r, 512)], xt_ref.at[:, pl.ds(512 * r, 512)],
                                  sems.at[r]) for r in range(4)]
    cp_bc = [pltpu.make_async_copy(w, bc_buf.at[j], sems.at[4 + j])
             for j, w in enumerate((bre_hbm, bim_hbm, cre_hbm, cim_hbm))]
    cp_q = wcopies(wq_hbm, wq_buf, 8)
    rest = ([pltpu.make_async_copy(c_hbm.at[0], c_ref, sems.at[10])]
            + wcopies(wk_hbm, wk_buf, 11) + wcopies(wv_hbm, wv_buf, 13)
            + [pltpu.make_async_copy(wo_hbm, wo_buf, sems.at[15])])
    for cp in (cp_x[0], cp_bc[0], cp_bc[1]):
        cp.start()

    def pre_u(r):
        if r == 0:
            for cp in (cp_x[0], cp_bc[0], cp_bc[1]):
                cp.wait()
            for cp in cp_x[1:]:
                cp.start()
        else:
            cp_x[r].wait()
        if r == 1:
            for cp in cp_q:
                cp.start()

    def pre_q():
        for cp in cp_q:
            cp.wait()
        for cp in cp_bc[2:] + rest[:3]:
            cp.start()

    def pre_y():
        cp_bc[2].wait()
        cp_bc[3].wait()

    def pre_2():
        rest[0].wait()
        for cp in rest[3:]:
            cp.start()

    def qproj(p):
        HS = S // 2
        blocks = []
        for r0, n in ((0, 256), (256, M - 256)):
            for j in range(2):
                w = wq_buf[j, pl.ds(p + 8 * r0, n, stride=8), :]
                v = jnp.concatenate([_lo16(w), _hi16(w)], axis=1)
                if n < 256:
                    v = jnp.concatenate([v, jnp.zeros((256 - n, 256), F32)], axis=0)
                blocks.append(v)

        def put(r, c, v):
            v = (v * (LOG2E / 16.0)).astype(BF16)
            for e in range(2):
                q_s[2 * p + e, pl.ds(r * HS, HS), pl.ds(c * 128, 128)] = v[:, e * 128:(e + 1) * 128]

        _strassen(xs_ref, rsx_ref, dx_ref, *blocks, put)

    _ssm(xt_ref, x_ref, lre_ref, lim_ref, bc_buf.at[0], bc_buf.at[1], bc_buf.at[2], bc_buf.at[3],
         ldt_ref, dsk_ref, gw_ref, acc_ref, g_ref, hre_ref, him_ref, pre_u, pre_y, pre_q, qproj, pre_2,
         c_ref, (xs_ref, rsx_ref, dx_ref), (cs_ref, rsc_ref, dc_ref))
    for cp in rest[1:]:
        cp.wait()

    def ocopy(i):
        cols = pl.ds(i * BQ, BQ)
        return pltpu.make_async_copy(acc_ref.at[:, cols], o_hbm.at[0, :, cols], osem.at[i])

    def kvproj(i, carry):
        HS, HK = S // 2, DC // 2
        for buf, dst in ((wk_buf, k_s), (wv_buf, v_s)):
            w = [buf[j, pl.ds(i + 8 * HK * r, HK, stride=8), :] for r in range(2) for j in range(2)]
            for e, f in enumerate((_lo16, _hi16)):
                def put(r, c, v, hh=2 * i + e, dst=dst):
                    dst[hh, pl.ds(r * HS, HS), pl.ds(c * 128, 128)] = v.astype(BF16)
                _strassen(cs_ref, rsc_ref, dc_ref, *[f(v) for v in w], put)
        return carry

    jax.lax.fori_loop(0, H // 2, kvproj, 0)

    def head(h, carry):
        NB = S // BQ
        HB = BQ // 2

        def tri(n):
            ri = jax.lax.broadcasted_iota(jnp.int32, (n, n), 0)
            ci = jax.lax.broadcasted_iota(jnp.int32, (n, n), 1)
            return ci <= ri

        def pv(b, s):
            p = jnp.exp2(s - jnp.max(s, axis=1, keepdims=True))
            sc = g_ref[pl.ds(b * HB, HB), :] * (1.0 / jnp.sum(p, axis=1, keepdims=True))
            c = _dot(p.astype(BF16), v_s[h, pl.ds(0, (b + 1) * HB), :])
            return (c * _rep(sc, D)).astype(BF16)

        def out(i, ctx):
            acc_ref[:, pl.ds(i * BQ, BQ)] += _dot_nt(wo_buf[h], ctx)

        def qkb(b):
            s = _dot_nt(q_s[h, pl.ds(b * HB, HB), :], k_s[h, pl.ds(0, (b + 1) * HB), :])
            sd = jnp.where(tri(HB), s[:, -HB:], -1e9)
            return sd if b == 0 else jnp.concatenate([s[:, :-HB], sd], axis=1)

        def outb(n):
            out(ORD[n], jnp.concatenate(cs[2 * n:2 * n + 2], axis=0))

            @pl.when(h == H - 1)
            def _():
                ocopy(ORD[n]).start()

        def out_prev():
            acc_ref[:, pl.ds(ORD[-1] * BQ, BQ)] += _dot_nt(wo_buf[jnp.maximum(h - 1, 0)], ctx_s[...])

        bs = [2 * i + e for i in ORD for e in range(2)]
        cs = []
        ss = [qkb(b) for b in bs[:AH]]
        out_prev()
        for n, b in enumerate(bs):
            if n + AH < len(bs):
                ss.append(qkb(bs[n + AH]))
            cs.append(pv(b, ss[n]))
            if n % 2 == 1 and n > 1:
                outb(n // 2 - 1)
        c = jnp.concatenate(cs[-2:], axis=0)
        ctx_s[...] = c
        return carry

    ctx_s[...] = jnp.zeros((BQ, D), BF16)
    jax.lax.fori_loop(0, H, head, 0)
    acc_ref[:, pl.ds(ORD[-1] * BQ, BQ)] += _dot_nt(wo_buf[H - 1], ctx_s[...])
    ocopy(ORD[-1]).start()
    for i in range(S // BQ):
        ocopy(i).wait()


BQ = 256
AH = 2
ORD = (1, 2, 3, 4, 5, 6, 7, 0)


@jax.jit
def pallas_gated_mix__compressed_kv_cla__ssm_conv_s5__prompt_kernel(
      A_x, A_c_kv, A_w_q, A_w_uk, A_w_uv, A_w_o, B_x, B_Lambda_re, B_Lambda_im, B_B_re, B_B_im,
      B_C_re, B_C_im, B_log_dt, B_Dskip, gate_w):
    del B_x
    vm = pl.BlockSpec(memory_space=pltpu.VMEM)
    hbm = pl.BlockSpec(memory_space=pltpu.HBM)
    out = pl.pallas_call(
        _kernel,
        in_specs=[hbm] * 10 + [vm] * 5,
        out_specs=hbm,
        out_shape=jax.ShapeDtypeStruct((1, M, S), F32),
        scratch_shapes=[
            pltpu.VMEM((M, S), BF16),
            pltpu.VMEM((S, 512), BF16),
            pltpu.VMEM((S, DC), BF16),
            pltpu.VMEM((2, M * 8, 128), U32),
            pltpu.VMEM((2, DC * 8, 128), U32),
            pltpu.VMEM((2, DC * 8, 128), U32),
            pltpu.VMEM((H, M, D), BF16),
            pltpu.VMEM((4, M, M), BF16),
            pltpu.SemaphoreType.DMA((16,)),
            pltpu.SemaphoreType.DMA((S // BQ,)),
            pltpu.VMEM((H, S, D), BF16),
            pltpu.VMEM((H, S, D), BF16),
            pltpu.VMEM((H, S, D), BF16),
            pltpu.VMEM((BQ, D), BF16),
            pltpu.VMEM((7, S // 2, DC // 2), BF16),
            pltpu.VMEM((7, S // 2, 256), BF16),
            pltpu.VMEM((S, 128), F32),
            pltpu.VMEM((S, 128), F32),
            pltpu.VMEM((DC, 128), F32),
            pltpu.VMEM((512, 128), F32),
            pltpu.VMEM((M, S), F32),
            pltpu.VMEM((S, 128), F32),
            pltpu.VMEM((4, NCH * PITCH, 128), F32),
            pltpu.VMEM((4, NCH * PITCH, 128), F32),
        ],
        compiler_params=pltpu.CompilerParams(vmem_limit_bytes=124 * 1024 * 1024),
    )(jnp.swapaxes(A_x, 1, 2), A_c_kv, A_w_q.reshape(M * H, D), A_w_uk.reshape(DC * H, D),
      A_w_uv.reshape(DC * H, D), jnp.swapaxes(A_w_o, 1, 2),
      B_B_re, B_B_im, B_C_re, B_C_im, B_Lambda_re, B_Lambda_im, B_log_dt, B_Dskip, gate_w)
    return jnp.swapaxes(out, 1, 2)
```
